```python
import jax
import jax.numpy as jnp

def _softmax(x, axis=-1):
    return jax.nn.softmax(x, axis=axis)

def _gelu(x):
    return jax.nn.gelu(x, approximate=True)

def _silu(x):
    return jax.nn.silu(x)

def _sigmoid(x):
    return jax.nn.sigmoid(x)

def _layernorm(x, axis=-1, eps=1e-05):
    m = jnp.mean(x, axis=axis, keepdims=True)
    v = jnp.var(x, axis=axis, keepdims=True)
    return (x - m) / jnp.sqrt(v + eps)

def _scatter_add(tgt, idx, src, axis=0):
    return tgt.at[idx].add(src)

def _segment_sum(src, seg, n):
    return jax.ops.segment_sum(src, seg, n)

class _Rng:

    def __init__(self, key):
        self._k = key

    def _next(self):
        self._k, sub = jax.random.split(self._k)
        return sub

    def normal(self, shape):
        return jax.random.normal(self._next(), shape, dtype=jnp.bfloat16)

    def randint(self, lo, hi, shape):
        return jax.random.randint(self._next(), shape, lo, hi, dtype=jnp.int32)

    def uniform(self, shape, lo=0.0, hi=1.0):
        return jax.random.uniform(self._next(), shape, jnp.bfloat16, lo, hi)

    def permutation(self, n):
        return jax.random.permutation(self._next(), n)
kernel_name = 'interleave_layers__memory_aug_recurrent_mem_tr__mixer_s_mlp__prompt'

def setup_inputs():
    _rng = _Rng(jax.random.key(int.from_bytes(__import__("os").urandom(4), "little")))
    _w = lambda a: (lambda t: t.astype(jnp.bfloat16) if jnp.issubdtype(t.dtype, jnp.floating) else t)(jnp.asarray(a))

    def _A_setup():
        B, S, Dm = (1, 2048, 640)
        H, Dh = (32, 192)
        M, seg = (8, 32)
        seg = min(seg, S)
        S = S // seg * seg
        return {'x': _w((lambda *s: _rng.normal(s) * 0.05)(B, S, Dm)), 'mem0': _w((lambda *s: _rng.normal(s) * 0.05)(B, M, Dm)), 'Wq': _w((lambda *s: _rng.normal(s) * 0.05)(Dm, H, Dh) * Dm ** (-0.5)), 'Wk': _w((lambda *s: _rng.normal(s) * 0.05)(Dm, H, Dh) * Dm ** (-0.5)), 'Wv': _w((lambda *s: _rng.normal(s) * 0.05)(Dm, H, Dh) * Dm ** (-0.5)), 'Wo': _w((lambda *s: _rng.normal(s) * 0.05)(H, Dh, Dm) * (H * Dh) ** (-0.5)), 'seg_len': seg}
    _A_in = _A_setup()

    def _B_setup():
        B, S, D, F = (1, 2048, 640, 1536)
        return {'x': _w((lambda *s: _rng.normal(s) * 0.05)(B, S, D)), 'w1': _w((lambda *s: _rng.normal(s) * 0.05)(D, D) * D ** (-0.5)), 'w2': _w((lambda *s: _rng.normal(s) * 0.05)(D, D) * D ** (-0.5)), 'w3': _w((lambda *s: _rng.normal(s) * 0.05)(D, F) * D ** (-0.5)), 'w4': _w((lambda *s: _rng.normal(s) * 0.05)(F, D) * F ** (-0.5))}
    _B_in = _B_setup()
    return {'A_x': _A_in['x'], 'A_mem0': _A_in['mem0'], 'A_Wq': _A_in['Wq'], 'A_Wk': _A_in['Wk'], 'A_Wv': _A_in['Wv'], 'A_Wo': _A_in['Wo'], 'A_seg_len': _A_in['seg_len'], 'B_x': _B_in['x'], 'B_w1': _B_in['w1'], 'B_w2': _B_in['w2'], 'B_w3': _B_in['w3'], 'B_w4': _B_in['w4']}

def reference(A_x, A_mem0, A_Wq, A_Wk, A_Wv, A_Wo, A_seg_len, B_x, B_w1, B_w2, B_w3, B_w4):

    def _A_ref(x, mem0, Wq, Wk, Wv, Wo, seg_len):
        B, S, Dm = x.shape
        H, Dh = (Wq.shape[1], Wq.shape[2])
        M = mem0.shape[1]
        scale = Dh ** (-0.5)
        n_seg = S // seg_len
        L = M + seg_len
        idx = jnp.arange(L)
        mask = (idx[:, None] < M) | (idx[:, None] >= idx[None, :])
        mem = mem0
        outs = []
        for s in range(n_seg):
            xs = x[:, s * seg_len:(s + 1) * seg_len, :].copy()
            h = jnp.concatenate([mem, xs], axis=1)
            q = jnp.einsum('btd,dhe->bhte', h, Wq)
            k = jnp.einsum('btd,dhe->bhte', h, Wk)
            v = jnp.einsum('btd,dhe->bhte', h, Wv)
            scores = jnp.einsum('bhqe,bhke->bhqk', q, k) * scale
            scores = jnp.where(mask[None, None], scores, -1000000000.0)
            p = _softmax(scores, axis=-1)
            o = jnp.einsum('bhqk,bhke->bhqe', p, v)
            o = jnp.einsum('bhte,hed->btd', o, Wo)
            mem = o[:, :M, :].copy()
            outs.append(o[:, M:, :])
        return jnp.concatenate(outs, axis=1)

    def _B_ref(x, w1, w2, w3, w4):
        B, S, D = x.shape
        h = _gelu(_layernorm(x, axis=-1) @ w1)
        c = D // 4
        g0 = jnp.pad(h[:, :, 0 * c:1 * c], ((0, 0), (1, 0), (0, 0)))[:, :S, :]
        g1 = jnp.pad(h[:, :, 1 * c:2 * c], ((0, 0), (0, 1), (0, 0)))[:, 1:, :]
        g2 = jnp.pad(h[:, :, 2 * c:3 * c], ((0, 0), (2, 0), (0, 0)))[:, :S, :]
        g3 = jnp.pad(h[:, :, 3 * c:], ((0, 0), (0, 2), (0, 0)))[:, 2:, :]
        hs = jnp.concatenate([g0, g1, g2, g3], axis=-1) @ w2
        x1 = x + hs
        h2 = _gelu(_layernorm(x1, axis=-1) @ w3) @ w4
        return x1 + h2
    x = A_x
    x = x + _A_ref(_layernorm(x, axis=-1), A_mem0, A_Wq, A_Wk, A_Wv, A_Wo, A_seg_len)
    x = x + _B_ref(_layernorm(x, axis=-1), B_w1, B_w2, B_w3, B_w4)
    x = x + _A_ref(_layernorm(x, axis=-1), A_mem0, A_Wq, A_Wk, A_Wv, A_Wo, A_seg_len)
    x = x + _B_ref(_layernorm(x, axis=-1), B_w1, B_w2, B_w3, B_w4)
    return x
```

```python
import functools

import jax
import jax.numpy as jnp
import jax.experimental.pallas as pl
import jax.experimental.pallas.tpu as pltpu

F32 = jnp.float32
BF16 = jnp.bfloat16

S, D, H, DH, M, SEG, FF = 2048, 640, 32, 192, 8, 32, 1536
NSEG = S // SEG
L = M + SEG
NPAIR = H // 2
PW = 2 * DH
QW = 3 * PW
LAG = 3
RING = 4
ZSLOT, TSLOT = RING, RING + 1
NSLOT = RING + 2
HALO = 8
EPS = 1e-5
SCALE = DH ** (-0.5)
NT = (((1,), (1,)), ((), ()))
DT = D // 128
KPRE = 8
NPRE = KPRE + LAG
RPRE = KPRE * SEG

PIPE = (1, 2, 3, 4)
ORDER = (0, 1, 2, 3, 4)
BPOS = (1, 5, 9, 13)
PUNROLL = 1


def _ln(x):
    m = jnp.mean(x, axis=-1, keepdims=True)
    xc = x - m
    v = jnp.mean(xc * xc, axis=-1, keepdims=True)
    return xc * jax.lax.rsqrt(v + EPS)


def _gelu(x):
    return jax.nn.gelu(x, approximate=True)


def _cat(xs, axis=0):
    return xs[0] if len(xs) == 1 else jnp.concatenate(xs, axis=axis)


def _lhs(x):
    return x.astype(BF16) if x.shape[0] % 16 == 0 else x


def _blockdiag(a):
    lane = jax.lax.broadcasted_iota(jnp.int32, (L, 128), 1)
    lo = lane < (DH - 128)
    a0, a1, a2 = a[:, 0:128], a[:, 128:256], a[:, 256:384]
    z = jnp.zeros_like(a0)
    top = jnp.concatenate([a0, jnp.where(lo, a1, 0.0), z], axis=1)
    bot = jnp.concatenate([z, jnp.where(lo, 0.0, a1), a2], axis=1)
    return jnp.concatenate([top, bot], axis=0).astype(BF16)


def _scores(q, k):
    return jax.lax.dot_general(q, _blockdiag(k), NT, preferred_element_type=F32)


def _softmax(s):
    lane = jax.lax.broadcasted_iota(jnp.int32, (L, 2 * L), 1)
    row = jax.lax.broadcasted_iota(jnp.int32, (L, 2 * L), 0)
    h0 = lane < L
    key = jnp.where(h0, lane, lane - L)
    mask = (row < M) | (row >= key)
    s = jnp.where(mask, s * SCALE, -1e9)
    ninf = -jnp.inf
    m0 = jnp.max(jnp.where(h0, s, ninf), axis=-1, keepdims=True)
    m1 = jnp.max(jnp.where(h0, ninf, s), axis=-1, keepdims=True)
    e = jnp.exp(s - jnp.where(h0, m0, m1))
    l0 = jnp.sum(jnp.where(h0, e, 0.0), axis=-1, keepdims=True)
    l1 = jnp.sum(jnp.where(h0, 0.0, e), axis=-1, keepdims=True)
    return e / jnp.where(h0, l0, l1)


def _pv(p, v):
    return jnp.dot(p, _blockdiag(v), preferred_element_type=F32)


def inner_kernel(x_hbm, mem0_ref, wq_hbm, wk_hbm, wv_hbm, wo_hbm,
                 w1_hbm, w2_hbm, w3_hbm, w4_hbm,
                 out_hbm,
                 wtq, wtk, wtv, wn, wo, w1, w2, w3, w4,
                 x0, lp, pre, x1, x2, x3, z1, z2, h1, h2, mem, obuf,
                 qsem, sems, osem):

    def qkv_copies(p):
        r = pl.ds(pl.multiple_of(p * PW, 128) if not isinstance(p, int) else p * PW, PW)
        return [pltpu.make_async_copy(a.at[r, :], b.at[r, :], qsem.at[p])
                for a, b in ((wq_hbm, wtq), (wk_hbm, wtk), (wv_hbm, wtv))]

    xh = pltpu.make_async_copy(x_hbm.at[pl.ds(0, NPRE * SEG), :], x0.at[pl.ds(0, NPRE * SEG), :],
                               sems.at[0])
    xt = pltpu.make_async_copy(x_hbm.at[pl.ds(NPRE * SEG, S - NPRE * SEG), :],
                               x0.at[pl.ds(NPRE * SEG, S - NPRE * SEG), :], sems.at[1])
    woc = pltpu.make_async_copy(wo_hbm, wo, sems.at[2])
    bcs = [pltpu.make_async_copy(a, b, sems.at[3 + i])
           for i, (a, b) in enumerate(((w1_hbm, w1), (w2_hbm, w2), (w3_hbm, w3), (w4_hbm, w4)))]
    def wo_copy(p):
        r = pl.ds(pl.multiple_of(p * PW, 128) if not isinstance(p, int) else p * PW, PW)
        return pltpu.make_async_copy(wo_hbm.at[r, :], wo.at[r, :], sems.at[2])

    def b_copy(j, i):
        a, b = ((w1_hbm, w1), (w2_hbm, w2), (w3_hbm, w3), (w4_hbm, w4))[j]
        n = b.shape[0] // 4
        r = pl.ds(pl.multiple_of(i * n, 16) if not isinstance(i, int) else i * n, n)
        return pltpu.make_async_copy(a.at[r, :], b.at[r, :], sems.at[3 + j])

    with jax.named_scope("dmastart"):
        xh.start()
        for c in qkv_copies(0):
            c.start()

    for b in (x1, x2, x3, z1, z2, h1, h2):
        b[...] = jnp.zeros(b.shape, F32)
    m0 = mem0_ref[...].astype(F32)
    mem[pl.ds(0, M), :] = m0
    mem[pl.ds(M, M), :] = m0
    eye = (jax.lax.broadcasted_iota(jnp.int32, (128, 128), 0)
           == jax.lax.broadcasted_iota(jnp.int32, (128, 128), 1)).astype(BF16)
    for kt in range(DT):
        lp[kt, pl.ds(RPRE, 128), :] = eye
    with jax.named_scope("xwait"):
      xh.wait()
    for c in qkv_copies(1):
        c.start()
    wo_copy(0).start()
    b_copy(0, 0).start()
    upre = _ln(x0[pl.ds(0, RPRE), :].astype(F32)).astype(BF16)
    for kt in range(DT):
        lp[kt, pl.ds(0, RPRE), :] = upre[:, kt * 128:(kt + 1) * 128]

    def pre_body(p, c):
        for cp in qkv_copies(p):
            cp.wait()

        @pl.when(p + 2 < NPAIR)
        def _():
            for cp in qkv_copies(p + 2):
                cp.start()

        @pl.when(p + 1 < NPAIR)
        def _():
            wo_copy(p + 1).start()
        for j in range(4):
            @pl.when((p + 1 < NPAIR) & ((p + 1) // 4 == j))
            def _():
                b_copy(j, (p + 1) % 4).start()
        r = pl.ds(pl.multiple_of(p * PW, 128), PW)
        acc = None
        for kt in range(DT):
            cols = pl.ds(kt * 128, 128)
            w = jnp.concatenate([wtq[r, cols], wtk[r, cols], wtv[r, cols]], axis=0)
            y = jax.lax.dot_general(lp[kt], w, NT, preferred_element_type=F32)
            wn[p, pl.ds(kt * 128, 128), :] = y[RPRE:].astype(BF16)
            acc = y[:RPRE] if acc is None else acc + y[:RPRE]
        pre[p, pl.ds(0, RPRE), :] = acc.astype(BF16)
        return c

    with jax.named_scope("prephase"):
        jax.lax.fori_loop(0, NPAIR, pre_body, 0, unroll=PUNROLL)
    with jax.named_scope("dmawait"):
        xt.start()
        woc.wait()
        for c in bcs:
            c.wait()

    def rows(slot):
        return pl.ds(pl.multiple_of(slot * SEG, SEG), SEG)

    def valid(s):
        return (s >= 0) & (s < NSEG)

    def rslot(s):
        return jnp.where(valid(s), s & (RING - 1), ZSLOT)

    def wslot(s):
        return jnp.where(valid(s), s & (RING - 1), TSLOT)

    def shift_mix(win):
        lane = jax.lax.broadcasted_iota(jnp.int32, (SEG, 128), 1)

        def sh(tile, off):
            return win[HALO + off:HALO + off + SEG, tile * 128:(tile + 1) * 128]
        t0 = sh(0, -1)
        t1 = jnp.where(lane < 32, sh(1, -1), sh(1, 1))
        t2 = jnp.where(lane < 64, sh(2, 1), sh(2, -2))
        t3 = jnp.where(lane < 96, sh(3, -2), sh(3, 2))
        t4 = sh(4, 2)
        return jnp.concatenate([t0, t1, t2, t3, t4], axis=1)

    def a_stage(t, a1, a2, stores):
        hs, res = [], []
        if a1:
            xa = x0[rows(t), :].astype(F32)
            hs.append(mem[pl.ds(0, M), :])
            if a1 == "now":
                hs.append(_ln(xa))
            elif a1 == "ahead":
                hs.append(_ln(x0[rows(t + NPRE - LAG), :].astype(F32)))
            res.append(xa)
        o2 = sum(a.shape[0] for a in hs)
        if a2:
            xb = x2[rows(rslot(t - LAG)), :]
            hs += [mem[pl.ds(M, M), :], _ln(xb)]
            res.append(xb)
        n = len(res)
        h = _lhs(_cat(hs))
        acc = None
        y, s, pr, o = {}, {}, {}, {}
        d1, d2, d3, d4 = PIPE

        def qkv(p, j):
            out = []
            c0, c1 = j * PW, (j + 1) * PW
            if a1 == "now":
                out.append(y[p][0:L, c0:c1])
            elif a1:
                tok = pre[p, rows(t), pl.ds(c0, PW)].astype(F32)
                out.append(jnp.concatenate([y[p][0:M, c0:c1], tok], axis=0))
            if a2:
                out.append(y[p][o2:o2 + L, c0:c1])
            return out

        for j in range(NPAIR + d4):
            for st in ORDER:
                if st == 0 and j < NPAIR:
                    y[j] = jnp.dot(h, wn[j], preferred_element_type=F32)
                    if a1 == "ahead":
                        stores.append((pre, (j, rows(t + NPRE - LAG)), y[j][M:L].astype(BF16)))
                p = j - d1
                if st == 1 and 0 <= p < NPAIR:
                    s[p] = [_scores(q, k) for q, k in zip(qkv(p, 0), qkv(p, 1))]
                p = j - d2
                if st == 2 and 0 <= p < NPAIR:
                    pr[p] = [_softmax(a) for a in s.pop(p)]
                p = j - d3
                if st == 3 and 0 <= p < NPAIR:
                    o[p] = _cat([_pv(a, v) for a, v in zip(pr.pop(p), qkv(p, 2))])
                    y.pop(p)
                p = j - d4
                if st == 4 and 0 <= p < NPAIR:
                    d = jnp.dot(_lhs(o.pop(p)), wo[pl.ds(p * PW, PW), :], preferred_element_type=F32)
                    acc = d if acc is None else acc + d
            yield
        outs = []
        for i in range(n):
            outs.append((acc[i * L:i * L + M], res[i] + acc[i * L + M:(i + 1) * L]))
        if a1:
            stores.append((mem, (pl.ds(0, M),), outs[0][0]))
            stores.append((x1, (rows(t & (RING - 1)),), outs[0][1]))
        if a2:
            stores.append((mem, (pl.ds(M, M),), outs[-1][0]))
            stores.append((x3, (rows((t - LAG) & (RING - 1)),), outs[-1][1]))

    def bb_chain(sh, zz, xres):
        g = jnp.dot(_lhs(_cat(sh)), w2[...], preferred_element_type=F32)
        yield
        y1 = _cat(zz) + g
        g = jnp.dot(_lhs(_ln(y1)), w3[...], preferred_element_type=F32)
        yield
        g = jnp.dot(_lhs(_gelu(g)), w4[...], preferred_element_type=F32)
        yield
        yield _cat(xres) + (y1 + g)

    def prev_tail(href, s):
        return href[pl.ds(pl.multiple_of(rslot(s - 1) * SEG + SEG - HALO, HALO), HALO), :]

    def b_stage(t, b1, b2, stores):
        lay = []
        if b1:
            lay.append((x1, z1, h1, t - 1, x2))
        if b2:
            lay.append((x3, z2, h2, t - 1 - LAG, None))
        if not lay:
            return
        xin = _cat([l[0][rows(rslot(l[3])), :] for l in lay])
        z = _ln(xin)
        g = jnp.dot(_lhs(_ln(z)), w1[...], preferred_element_type=F32)
        yield
        hh = _gelu(g)
        head = []
        for i, l in enumerate(lay):
            s = l[3]
            hi = jnp.where(valid(s), hh[i * SEG:(i + 1) * SEG], 0.0)
            head.append(hi[0:HALO])
            stores.append((l[1], (rows(wslot(s)),), z[i * SEG:(i + 1) * SEG]))
            stores.append((l[2], (rows(wslot(s)),), hi))
        sh, zz, xres = [], [], []
        for i, l in enumerate(lay):
            s = l[3] - 1
            win = jnp.concatenate([prev_tail(l[2], s), l[2][rows(rslot(s)), :], head[i]], axis=0)
            sh.append(shift_mix(win))
            zz.append(l[1][rows(rslot(s)), :])
            xres.append(l[0][rows(rslot(s)), :])
        chain = bb_chain(sh, zz, xres)
        next(chain)
        yield
        next(chain)
        yield
        next(chain)
        yield
        xn = next(chain)
        for i, l in enumerate(lay):
            s = l[3] - 1
            v = xn[i * SEG:(i + 1) * SEG]
            if l[4] is not None:
                stores.append((l[4], (rows(wslot(s)),), v))
            else:
                so = jnp.where(valid(s), s, NSEG)
                stores.append((obuf, (rows(so),), v.astype(BF16)))

    def step(t, a1, a2, b1, b2):
        stores = []
        bg = b_stage(t, b1, b2, stores)
        if a1 or a2:
            ag = a_stage(t, a1, a2, stores)
            j = 0
            for _ in ag:
                if j in BPOS:
                    next(bg, None)
                j += 1
        for _ in bg:
            pass
        for ref, idx, val in stores:
            ref[idx + (slice(None),)] = val

    def loop(lo, hi, *flags):
        def body(t, c):
            step(t, *flags)
            return c
        with jax.named_scope("loop_%d_%d" % (lo, hi)):
            jax.lax.fori_loop(lo, hi, body, 0)

    T, Fa = True, False
    loop(0, LAG, "ahead", Fa, T, Fa)
    loop(LAG, NPRE, "pre", T, T, T)
    with jax.named_scope("xtwait"):
      xt.wait()
    loop(NPRE, NSEG, "now", T, T, T)
    done = NSEG - 5
    oc1 = pltpu.make_async_copy(obuf.at[pl.ds(0, done * SEG), :],
                                out_hbm.at[pl.ds(0, done * SEG), :], osem.at[0])
    oc1.start()
    loop(NSEG, NSEG + LAG, None, T, T, T)

    with jax.named_scope("tail"):
        sa, sb = NSEG - 1, NSEG - 2
        ra, rb, rc = [pl.ds((s % RING) * SEG, SEG) for s in (sa, sb, sb - 1)]
        xa = x3[ra, :]
        za = _ln(xa)
        ha = _gelu(jnp.dot(_lhs(_ln(za)), w1[...], preferred_element_type=F32))
        hb = h2[rb, :]
        winb = jnp.concatenate([h2[rc, :][SEG - HALO:], hb, ha[0:HALO]], axis=0)
        wina = jnp.concatenate([hb[SEG - HALO:], ha, jnp.zeros((HALO, D), F32)], axis=0)
        chain = bb_chain([shift_mix(winb), shift_mix(wina)], [z2[rb, :], za], [x3[rb, :], xa])
        next(chain), next(chain), next(chain)
        obuf[pl.ds(sb * SEG, 2 * SEG), :] = next(chain).astype(BF16)

    with jax.named_scope("outdma"):
        oc2 = pltpu.make_async_copy(obuf.at[pl.ds(done * SEG, S - done * SEG), :],
                                    out_hbm.at[pl.ds(done * SEG, S - done * SEG), :], osem.at[1])
        oc2.start()
        oc1.wait()
        oc2.wait()


@functools.partial(jax.jit, static_argnames=("A_seg_len",))
def pallas_interleave_layers__memory_aug_recurrent_mem_tr__mixer_s_mlp__prompt_kernel(
    A_x, A_mem0, A_Wq, A_Wk, A_Wv, A_Wo, A_seg_len, B_x, B_w1, B_w2, B_w3, B_w4,
):
    del B_x
    assert A_seg_len == SEG and A_x.shape == (1, S, D) and A_mem0.shape == (1, M, D)
    assert A_Wq.shape == (D, H, DH) and A_Wo.shape == (H, DH, D) and B_w3.shape == (D, FF)

    def wt(w):
        return jnp.transpose(w, (1, 2, 0)).reshape(H * DH, D)

    any_spec = pl.BlockSpec(memory_space=pl.ANY)
    out = pl.pallas_call(
        inner_kernel,
        out_shape=jax.ShapeDtypeStruct((S, D), BF16),
        in_specs=[any_spec, pl.BlockSpec(memory_space=pltpu.VMEM)] + [any_spec] * 8,
        out_specs=any_spec,
        scratch_shapes=[
            pltpu.VMEM((H * DH, D), BF16),
            pltpu.VMEM((H * DH, D), BF16),
            pltpu.VMEM((H * DH, D), BF16),
            pltpu.VMEM((NPAIR, D, QW), BF16),
            pltpu.VMEM((H * DH, D), BF16),
            pltpu.VMEM((D, D), BF16),
            pltpu.VMEM((D, D), BF16),
            pltpu.VMEM((D, FF), BF16),
            pltpu.VMEM((FF, D), BF16),
            pltpu.VMEM((S, D), BF16),
            pltpu.VMEM((DT, RPRE + 128, 128), BF16),
            pltpu.VMEM((NPAIR, NPRE * SEG, QW), BF16),
            pltpu.VMEM((NSLOT * SEG, D), F32),
            pltpu.VMEM((NSLOT * SEG, D), F32),
            pltpu.VMEM((NSLOT * SEG, D), F32),
            pltpu.VMEM((NSLOT * SEG, D), F32),
            pltpu.VMEM((NSLOT * SEG, D), F32),
            pltpu.VMEM((NSLOT * SEG, D), F32),
            pltpu.VMEM((NSLOT * SEG, D), F32),
            pltpu.VMEM((2 * M, D), F32),
            pltpu.VMEM((S + SEG, D), BF16),
            pltpu.SemaphoreType.DMA((NPAIR,)),
            pltpu.SemaphoreType.DMA((7,)),
            pltpu.SemaphoreType.DMA((2,)),
        ],
        compiler_params=pltpu.CompilerParams(vmem_limit_bytes=120 * 2**20),
    )(A_x.reshape(S, D), A_mem0.reshape(M, D), wt(A_Wq), wt(A_Wk), wt(A_Wv),
      A_Wo.reshape(H * DH, D), B_w1, B_w2, B_w3, B_w4)
    return out.reshape(1, S, D)
```

```python
import functools

import jax
import jax.numpy as jnp
import jax.experimental.pallas as pl
import jax.experimental.pallas.tpu as pltpu

F32 = jnp.float32
BF16 = jnp.bfloat16

S, D, H, DH, M, SEG, FF = 2048, 640, 32, 192, 8, 32, 1536
NSEG = S // SEG
L = M + SEG
NPAIR = H // 2
PW = 2 * DH
QW = 3 * PW
LAG = 3
RING = 4
ZSLOT, TSLOT = RING, RING + 1
NSLOT = RING + 2
HALO = 8
EPS = 1e-5
SCALE = DH ** (-0.5)
NT = (((1,), (1,)), ((), ()))
DT = D // 128
KPRE = 12
NPRE = KPRE + LAG
RPRE = KPRE * SEG

PIPE = (1, 2, 3, 4)
ORDER = (0, 1, 2, 3, 4)
BPOS = (1, 5, 9, 13)
PUNROLL = 1


def _ln(x):
    m = jnp.mean(x, axis=-1, keepdims=True)
    xc = x - m
    v = jnp.mean(xc * xc, axis=-1, keepdims=True)
    return xc * jax.lax.rsqrt(v + EPS)


def _gelu(x):
    return jax.nn.gelu(x, approximate=True)


def _cat(xs, axis=0):
    return xs[0] if len(xs) == 1 else jnp.concatenate(xs, axis=axis)


def _lhs(x):
    return x.astype(BF16) if x.shape[0] % 16 == 0 else x


def _blockdiag(a):
    lane = jax.lax.broadcasted_iota(jnp.int32, (L, 128), 1)
    lo = lane < (DH - 128)
    a0, a1, a2 = a[:, 0:128], a[:, 128:256], a[:, 256:384]
    z = jnp.zeros_like(a0)
    top = jnp.concatenate([a0, jnp.where(lo, a1, 0.0), z], axis=1)
    bot = jnp.concatenate([z, jnp.where(lo, 0.0, a1), a2], axis=1)
    return jnp.concatenate([top, bot], axis=0).astype(BF16)


def _scores(q, k):
    return jax.lax.dot_general(q, _blockdiag(k), NT, preferred_element_type=F32)


def _softmax(s):
    lane = jax.lax.broadcasted_iota(jnp.int32, (L, 2 * L), 1)
    row = jax.lax.broadcasted_iota(jnp.int32, (L, 2 * L), 0)
    h0 = lane < L
    key = jnp.where(h0, lane, lane - L)
    mask = (row < M) | (row >= key)
    s = jnp.where(mask, s * SCALE, -1e9)
    ninf = -jnp.inf
    m0 = jnp.max(jnp.where(h0, s, ninf), axis=-1, keepdims=True)
    m1 = jnp.max(jnp.where(h0, ninf, s), axis=-1, keepdims=True)
    e = jnp.exp(s - jnp.where(h0, m0, m1))
    l0 = jnp.sum(jnp.where(h0, e, 0.0), axis=-1, keepdims=True)
    l1 = jnp.sum(jnp.where(h0, 0.0, e), axis=-1, keepdims=True)
    return e / jnp.where(h0, l0, l1)


def _pv(p, v):
    return jnp.dot(p, _blockdiag(v), preferred_element_type=F32)


def inner_kernel(x_hbm, mem0_ref, wq_hbm, wk_hbm, wv_hbm, wo_hbm,
                 w1_hbm, w2_hbm, w3_hbm, w4_hbm,
                 out_hbm,
                 wtq, wtk, wtv, wn, wo, w1, w2, w3, w4,
                 x0, lp, ub, pre, x1, x2, x3, z1, z2, h1, h2, mem, obuf,
                 qsem, sems, osem):

    def qkv_copies(p):
        r = pl.ds(pl.multiple_of(p * PW, 128) if not isinstance(p, int) else p * PW, PW)
        return [pltpu.make_async_copy(a.at[r, :], b.at[r, :], qsem.at[p])
                for a, b in ((wq_hbm, wtq), (wk_hbm, wtk), (wv_hbm, wtv))]

    xh = pltpu.make_async_copy(x_hbm.at[pl.ds(0, NPRE * SEG), :], x0.at[pl.ds(0, NPRE * SEG), :],
                               sems.at[0])
    xt = pltpu.make_async_copy(x_hbm.at[pl.ds(NPRE * SEG, S - NPRE * SEG), :],
                               x0.at[pl.ds(NPRE * SEG, S - NPRE * SEG), :], sems.at[1])
    woc = pltpu.make_async_copy(wo_hbm, wo, sems.at[2])
    bcs = [pltpu.make_async_copy(a, b, sems.at[3 + i])
           for i, (a, b) in enumerate(((w1_hbm, w1), (w2_hbm, w2), (w3_hbm, w3), (w4_hbm, w4)))]
    def wo_copy(p):
        r = pl.ds(pl.multiple_of(p * PW, 128) if not isinstance(p, int) else p * PW, PW)
        return pltpu.make_async_copy(wo_hbm.at[r, :], wo.at[r, :], sems.at[2])

    def b_copy(j, i):
        a, b = ((w1_hbm, w1), (w2_hbm, w2), (w3_hbm, w3), (w4_hbm, w4))[j]
        n = b.shape[0] // 4
        r = pl.ds(pl.multiple_of(i * n, 16) if not isinstance(i, int) else i * n, n)
        return pltpu.make_async_copy(a.at[r, :], b.at[r, :], sems.at[3 + j])

    with jax.named_scope("dmastart"):
        xh.start()
        for c in qkv_copies(0):
            c.start()

    for b in (x1, x2, x3, z1, z2, h1, h2):
        b[...] = jnp.zeros(b.shape, F32)
    ub[...] = jnp.zeros(ub.shape, BF16)
    m0 = mem0_ref[...].astype(F32)
    mem[pl.ds(0, M), :] = m0
    mem[pl.ds(M, M), :] = m0
    with jax.named_scope("xwait"):
      xh.wait()
    for c in qkv_copies(1):
        c.start()
    wo_copy(0).start()
    b_copy(0, 0).start()
    upre = _ln(x0[pl.ds(0, RPRE), :].astype(F32)).astype(BF16)
    lp[...] = upre

    def pre_body(p, c):
        for cp in qkv_copies(p):
            cp.wait()

        @pl.when(p + 2 < NPAIR)
        def _():
            for cp in qkv_copies(p + 2):
                cp.start()

        @pl.when(p + 1 < NPAIR)
        def _():
            wo_copy(p + 1).start()
        for j in range(4):
            @pl.when((p + 1 < NPAIR) & ((p + 1) // 4 == j))
            def _():
                b_copy(j, (p + 1) % 4).start()
        r = pl.ds(pl.multiple_of(p * PW, 128), PW)
        w = jnp.concatenate([wtq[r, :], wtk[r, :], wtv[r, :]], axis=0)
        wt = w.T
        for c_ in range(QW // 128):
            wn[p, c_, :, :] = wt[:, c_ * 128:(c_ + 1) * 128]
        y = jax.lax.dot_general(lp[...], w, NT, preferred_element_type=F32)
        pre[p, pl.ds(0, RPRE), :] = y.astype(BF16)
        return c

    with jax.named_scope("prephase"):
        jax.lax.fori_loop(0, NPAIR, pre_body, 0, unroll=PUNROLL)
    with jax.named_scope("dmawait"):
        xt.start()
        woc.wait()
        for c in bcs:
            c.wait()

    def rows(slot):
        return pl.ds(pl.multiple_of(slot * SEG, SEG), SEG)

    def valid(s):
        return (s >= 0) & (s < NSEG)

    def rslot(s):
        return jnp.where(valid(s), s & (RING - 1), ZSLOT)

    def wslot(s):
        return jnp.where(valid(s), s & (RING - 1), TSLOT)

    def shift_mix(win):
        lane = jax.lax.broadcasted_iota(jnp.int32, (SEG, 128), 1)

        def sh(tile, off):
            return win[HALO + off:HALO + off + SEG, tile * 128:(tile + 1) * 128]
        t0 = sh(0, -1)
        t1 = jnp.where(lane < 32, sh(1, -1), sh(1, 1))
        t2 = jnp.where(lane < 64, sh(2, 1), sh(2, -2))
        t3 = jnp.where(lane < 96, sh(3, -2), sh(3, 2))
        t4 = sh(4, 2)
        return jnp.concatenate([t0, t1, t2, t3, t4], axis=1)

    def ub_load(i):
        return jnp.concatenate([ub[c, pl.ds(i * SEG, SEG), :] for c in range(DT)], axis=1)

    def ub_store(i, val, stores):
        v = val.astype(BF16)
        for c in range(DT):
            stores.append((ub, (c, pl.ds(i * SEG, SEG)), v[:, c * 128:(c + 1) * 128]))

    def a_stage(t, a1, a2, stores):
        res, toks = [], []
        if a1:
            res.append(x0[rows(t), :].astype(F32))
            if a1 in ("now", "ahead"):
                toks.append(ub_load(0))
                nxt = jnp.minimum(t + 1, NSEG - 1) if a1 == "now" else jnp.minimum(
                    t + 1 + NPRE - LAG, NPRE - 1)
                ub_store(0, _ln(x0[rows(nxt), :].astype(F32)), stores)
        if a2:
            res.append(x2[rows(rslot(t - LAG)), :])
            toks.append(ub_load(1))
        if a1 and a2:
            h = jnp.concatenate([mem[...].astype(BF16)] + toks, axis=0)
            m1, m2, t1 = 0, M, 2 * M
            t2 = t1 + (SEG if a1 == "now" else 0)
        else:
            h = jnp.concatenate([mem[pl.ds(0 if a1 else M, M), :], toks[0].astype(F32)], axis=0)
            m1 = m2 = 0
            t1 = t2 = M
        n = len(res)
        acc = None
        y, s, pr, o = {}, {}, {}, {}
        d1, d2, d3, d4 = PIPE

        def qkv(p, j):
            out = []
            c0, c1 = j * PW, (j + 1) * PW
            if a1 == "now":
                out.append(jnp.concatenate([y[p][m1:m1 + M, c0:c1], y[p][t1:t1 + SEG, c0:c1]], axis=0))
            elif a1:
                tok = pre[p, rows(t), pl.ds(c0, PW)].astype(F32)
                out.append(jnp.concatenate([y[p][m1:m1 + M, c0:c1], tok], axis=0))
            if a2:
                out.append(jnp.concatenate([y[p][m2:m2 + M, c0:c1], y[p][t2:t2 + SEG, c0:c1]], axis=0))
            return out

        for j in range(NPAIR + d4):
            for st in ORDER:
                if st == 0 and j < NPAIR:
                    y[j] = jnp.dot(h, jnp.concatenate([wn[j, c] for c in range(QW // 128)], axis=1),
                                   preferred_element_type=F32)
                    if a1 == "ahead":
                        stores.append((pre, (j, rows(t + NPRE - LAG)), y[j][t1:t1 + SEG].astype(BF16)))
                p = j - d1
                if st == 1 and 0 <= p < NPAIR:
                    s[p] = [_scores(q, k) for q, k in zip(qkv(p, 0), qkv(p, 1))]
                p = j - d2
                if st == 2 and 0 <= p < NPAIR:
                    pr[p] = [_softmax(a) for a in s.pop(p)]
                p = j - d3
                if st == 3 and 0 <= p < NPAIR:
                    o[p] = _cat([_pv(a, v) for a, v in zip(pr.pop(p), qkv(p, 2))])
                    y.pop(p)
                p = j - d4
                if st == 4 and 0 <= p < NPAIR:
                    d = jnp.dot(_lhs(o.pop(p)), wo[pl.ds(p * PW, PW), :], preferred_element_type=F32)
                    acc = d if acc is None else acc + d
            yield
        outs = []
        for i in range(n):
            outs.append((acc[i * L:i * L + M], res[i] + acc[i * L + M:(i + 1) * L]))
        if a1:
            stores.append((mem, (pl.ds(0, M),), outs[0][0]))
            stores.append((x1, (rows(t & (RING - 1)),), outs[0][1]))
        if a2:
            stores.append((mem, (pl.ds(M, M),), outs[-1][0]))
            stores.append((x3, (rows((t - LAG) & (RING - 1)),), outs[-1][1]))

    def bb_chain(sh, zz, xres):
        g = jnp.dot(_lhs(_cat(sh)), w2[...], preferred_element_type=F32)
        yield
        y1 = _cat(zz) + g
        g = jnp.dot(_lhs(_ln(y1)), w3[...], preferred_element_type=F32)
        yield
        g = jnp.dot(_lhs(_gelu(g)), w4[...], preferred_element_type=F32)
        yield
        yield _cat(xres) + (y1 + g)

    def prev_tail(href, s):
        return href[pl.ds(pl.multiple_of(rslot(s - 1) * SEG + SEG - HALO, HALO), HALO), :]

    def b_stage(t, b1, b2, stores):
        lay = []
        if b1:
            lay.append((x1, z1, h1, t - 1, x2))
        if b2:
            lay.append((x3, z2, h2, t - 1 - LAG, None))
        if not lay:
            return
        xin = _cat([l[0][rows(rslot(l[3])), :] for l in lay])
        z = _ln(xin)
        g = jnp.dot(_lhs(_ln(z)), w1[...], preferred_element_type=F32)
        yield
        hh = _gelu(g)
        head = []
        for i, l in enumerate(lay):
            s = l[3]
            hi = jnp.where(valid(s), hh[i * SEG:(i + 1) * SEG], 0.0)
            head.append(hi[0:HALO])
            stores.append((l[1], (rows(wslot(s)),), z[i * SEG:(i + 1) * SEG]))
            stores.append((l[2], (rows(wslot(s)),), hi))
        sh, zz, xres = [], [], []
        for i, l in enumerate(lay):
            s = l[3] - 1
            win = jnp.concatenate([prev_tail(l[2], s), l[2][rows(rslot(s)), :], head[i]], axis=0)
            sh.append(shift_mix(win))
            zz.append(l[1][rows(rslot(s)), :])
            xres.append(l[0][rows(rslot(s)), :])
        chain = bb_chain(sh, zz, xres)
        next(chain)
        yield
        next(chain)
        yield
        next(chain)
        yield
        xn = next(chain)
        for i, l in enumerate(lay):
            s = l[3] - 1
            v = xn[i * SEG:(i + 1) * SEG]
            if l[4] is not None:
                stores.append((l[4], (rows(wslot(s)),), v))
                ub_store(1, _ln(v), stores)
            else:
                so = jnp.where(valid(s), s, NSEG)
                stores.append((obuf, (rows(so),), v.astype(BF16)))

    def step(t, a1, a2, b1, b2):
        stores = []
        bg = b_stage(t, b1, b2, stores)
        if a1 or a2:
            ag = a_stage(t, a1, a2, stores)
            j = 0
            for _ in ag:
                if j in BPOS:
                    next(bg, None)
                j += 1
        for _ in bg:
            pass
        for ref, idx, val in stores:
            ref[idx + (slice(None),)] = val

    def loop(lo, hi, *flags):
        def body(t, c):
            step(t, *flags)
            return c
        with jax.named_scope("loop_%d_%d" % (lo, hi)):
            jax.lax.fori_loop(lo, hi, body, 0)

    T, Fa = True, False

    def prefill(seg):
        st = []
        ub_store(0, _ln(x0[pl.ds(seg * SEG, SEG), :].astype(F32)), st)
        for ref, idx, val in st:
            ref[idx + (slice(None),)] = val

    prefill(NPRE - LAG)
    loop(0, LAG, "ahead", Fa, T, Fa)
    loop(LAG, NPRE, "pre", T, T, T)
    with jax.named_scope("xtwait"):
      xt.wait()
    prefill(NPRE)
    loop(NPRE, NSEG, "now", T, T, T)
    done = NSEG - 5
    oc1 = pltpu.make_async_copy(obuf.at[pl.ds(0, done * SEG), :],
                                out_hbm.at[pl.ds(0, done * SEG), :], osem.at[0])
    oc1.start()
    loop(NSEG, NSEG + LAG, None, T, T, T)

    with jax.named_scope("tail"):
        sa, sb = NSEG - 1, NSEG - 2
        ra, rb, rc = [pl.ds((s % RING) * SEG, SEG) for s in (sa, sb, sb - 1)]
        xa = x3[ra, :]
        za = _ln(xa)
        ha = _gelu(jnp.dot(_lhs(_ln(za)), w1[...], preferred_element_type=F32))
        hb = h2[rb, :]
        winb = jnp.concatenate([h2[rc, :][SEG - HALO:], hb, ha[0:HALO]], axis=0)
        wina = jnp.concatenate([hb[SEG - HALO:], ha, jnp.zeros((HALO, D), F32)], axis=0)
        chain = bb_chain([shift_mix(winb), shift_mix(wina)], [z2[rb, :], za], [x3[rb, :], xa])
        next(chain), next(chain), next(chain)
        obuf[pl.ds(sb * SEG, 2 * SEG), :] = next(chain).astype(BF16)

    with jax.named_scope("outdma"):
        oc2 = pltpu.make_async_copy(obuf.at[pl.ds(done * SEG, S - done * SEG), :],
                                    out_hbm.at[pl.ds(done * SEG, S - done * SEG), :], osem.at[1])
        oc2.start()
        oc1.wait()
        oc2.wait()


@functools.partial(jax.jit, static_argnames=("A_seg_len",))
def pallas_interleave_layers__memory_aug_recurrent_mem_tr__mixer_s_mlp__prompt_kernel(
    A_x, A_mem0, A_Wq, A_Wk, A_Wv, A_Wo, A_seg_len, B_x, B_w1, B_w2, B_w3, B_w4,
):
    del B_x
    assert A_seg_len == SEG and A_x.shape == (1, S, D) and A_mem0.shape == (1, M, D)
    assert A_Wq.shape == (D, H, DH) and A_Wo.shape == (H, DH, D) and B_w3.shape == (D, FF)

    def wt(w):
        return jnp.transpose(w, (1, 2, 0)).reshape(H * DH, D)

    any_spec = pl.BlockSpec(memory_space=pl.ANY)
    out = pl.pallas_call(
        inner_kernel,
        out_shape=jax.ShapeDtypeStruct((S, D), BF16),
        in_specs=[any_spec, pl.BlockSpec(memory_space=pltpu.VMEM)] + [any_spec] * 8,
        out_specs=any_spec,
        scratch_shapes=[
            pltpu.VMEM((H * DH, D), BF16),
            pltpu.VMEM((H * DH, D), BF16),
            pltpu.VMEM((H * DH, D), BF16),
            pltpu.VMEM((NPAIR, QW // 128, D, 128), BF16),
            pltpu.VMEM((H * DH, D), BF16),
            pltpu.VMEM((D, D), BF16),
            pltpu.VMEM((D, D), BF16),
            pltpu.VMEM((D, FF), BF16),
            pltpu.VMEM((FF, D), BF16),
            pltpu.VMEM((S, D), BF16),
            pltpu.VMEM((RPRE, D), BF16),
            pltpu.VMEM((DT, 2 * SEG, 128), BF16),
            pltpu.VMEM((NPAIR, NPRE * SEG, QW), BF16),
            pltpu.VMEM((NSLOT * SEG, D), F32),
            pltpu.VMEM((NSLOT * SEG, D), F32),
            pltpu.VMEM((NSLOT * SEG, D), F32),
            pltpu.VMEM((NSLOT * SEG, D), F32),
            pltpu.VMEM((NSLOT * SEG, D), F32),
            pltpu.VMEM((NSLOT * SEG, D), F32),
            pltpu.VMEM((NSLOT * SEG, D), F32),
            pltpu.VMEM((2 * M, D), F32),
            pltpu.VMEM((S + SEG, D), BF16),
            pltpu.SemaphoreType.DMA((NPAIR,)),
            pltpu.SemaphoreType.DMA((7,)),
            pltpu.SemaphoreType.DMA((2,)),
        ],
        compiler_params=pltpu.CompilerParams(vmem_limit_bytes=120 * 2**20),
    )(A_x.reshape(S, D), A_mem0.reshape(M, D), wt(A_Wq), wt(A_Wk), wt(A_Wv),
      A_Wo.reshape(H * DH, D), B_w1, B_w2, B_w3, B_w4)
    return out.reshape(1, S, D)
```

```python
import functools

import jax
import jax.numpy as jnp
import jax.experimental.pallas as pl
import jax.experimental.pallas.tpu as pltpu

F32 = jnp.float32
BF16 = jnp.bfloat16

S, D, H, DH, M, SEG, FF = 2048, 640, 32, 192, 8, 32, 1536
NSEG = S // SEG
L = M + SEG
NPAIR = H // 2
PW = 2 * DH
QW = 3 * PW
LAG = 3
RING = 4
ZSLOT, TSLOT = RING, RING + 1
NSLOT = RING + 2
HALO = 8
EPS = 1e-5
SCALE = DH ** (-0.5)
NT = (((1,), (1,)), ((), ()))
DT = D // 128
KPRE = 12
NPRE = KPRE + LAG
RPRE = KPRE * SEG

PIPE = (1, 2, 3, 4)
ORDER = (0, 1, 2, 3, 4)
BPOS0 = (4, 8, 12, 16)
BPOS1 = (4, 7, 10, 13)
BPOS2 = (2, 4, 7, 10)
BPOS3 = (10, 13, 15, 17)
EARLY = 0
NEARLY = 0
NLATE = 0
LATE = (0, 0, 0, 0, 0)
PUNROLL = 1


def _ln(x):
    m = jnp.mean(x, axis=-1, keepdims=True)
    xc = x - m
    v = jnp.mean(xc * xc, axis=-1, keepdims=True)
    return xc * jax.lax.rsqrt(v + EPS)


def _gelu(x):
    return jax.nn.gelu(x, approximate=True)


def _cat(xs, axis=0):
    return xs[0] if len(xs) == 1 else jnp.concatenate(xs, axis=axis)


def _lhs(x):
    return x.astype(BF16) if x.shape[0] % 16 == 0 else x


def _blockdiag(a):
    lane = jax.lax.broadcasted_iota(jnp.int32, (L, 128), 1)
    lo = lane < (DH - 128)
    a0, a1, a2 = a[:, 0:128], a[:, 128:256], a[:, 256:384]
    z = jnp.zeros_like(a0)
    top = jnp.concatenate([a0, jnp.where(lo, a1, 0.0), z], axis=1)
    bot = jnp.concatenate([z, jnp.where(lo, 0.0, a1), a2], axis=1)
    return jnp.concatenate([top, bot], axis=0).astype(BF16)


def _scores(q, k):
    return jax.lax.dot_general(q, _blockdiag(k), NT, preferred_element_type=F32)


def _softmax(s):
    lane = jax.lax.broadcasted_iota(jnp.int32, (L, 2 * L), 1)
    row = jax.lax.broadcasted_iota(jnp.int32, (L, 2 * L), 0)
    h0 = lane < L
    key = jnp.where(h0, lane, lane - L)
    mask = (row < M) | (row >= key)
    s = jnp.where(mask, s * SCALE, -1e9)
    ninf = -jnp.inf
    m0 = jnp.max(jnp.where(h0, s, ninf), axis=-1, keepdims=True)
    m1 = jnp.max(jnp.where(h0, ninf, s), axis=-1, keepdims=True)
    e = jnp.exp(s - jnp.where(h0, m0, m1))
    l0 = jnp.sum(jnp.where(h0, e, 0.0), axis=-1, keepdims=True)
    l1 = jnp.sum(jnp.where(h0, 0.0, e), axis=-1, keepdims=True)
    return e / jnp.where(h0, l0, l1)


def _pv(p, v):
    return jnp.dot(p, _blockdiag(v), preferred_element_type=F32)


def inner_kernel(x_hbm, mem0_ref, wq_hbm, wk_hbm, wv_hbm, wo_hbm,
                 w1_hbm, w2_hbm, w3_hbm, w4_hbm,
                 out_hbm,
                 wtq, wtk, wtv, wn, wo, w1, w2, w3, w4,
                 x0, lp, ub, pre, x1, x2, x3, z1, z2, h1, h2, mem, obuf,
                 qsem, sems, osem):

    def qkv_copies(p):
        r = pl.ds(pl.multiple_of(p * PW, 128) if not isinstance(p, int) else p * PW, PW)
        return [pltpu.make_async_copy(a.at[r, :], b.at[r, :], qsem.at[p])
                for a, b in ((wq_hbm, wtq), (wk_hbm, wtk), (wv_hbm, wtv))]

    xh = pltpu.make_async_copy(x_hbm.at[pl.ds(0, NPRE * SEG), :], x0.at[pl.ds(0, NPRE * SEG), :],
                               sems.at[0])
    xt = pltpu.make_async_copy(x_hbm.at[pl.ds(NPRE * SEG, S - NPRE * SEG), :],
                               x0.at[pl.ds(NPRE * SEG, S - NPRE * SEG), :], sems.at[1])
    woc = pltpu.make_async_copy(wo_hbm, wo, sems.at[2])
    bcs = [pltpu.make_async_copy(a, b, sems.at[3 + i])
           for i, (a, b) in enumerate(((w1_hbm, w1), (w2_hbm, w2), (w3_hbm, w3), (w4_hbm, w4)))]
    def wo_copy(p):
        r = pl.ds(pl.multiple_of(p * PW, 128) if not isinstance(p, int) else p * PW, PW)
        return pltpu.make_async_copy(wo_hbm.at[r, :], wo.at[r, :], sems.at[2])

    def b_copy(j, i):
        a, b = ((w1_hbm, w1), (w2_hbm, w2), (w3_hbm, w3), (w4_hbm, w4))[j]
        n = b.shape[0] // 4
        r = pl.ds(pl.multiple_of(i * n, 16) if not isinstance(i, int) else i * n, n)
        return pltpu.make_async_copy(a.at[r, :], b.at[r, :], sems.at[3 + j])

    with jax.named_scope("dmastart"):
        xh.start()
        for c in qkv_copies(0):
            c.start()

    for b in (x1, x2, x3, z1, z2, h1, h2):
        b[...] = jnp.zeros(b.shape, F32)
    ub[...] = jnp.zeros(ub.shape, BF16)
    m0 = mem0_ref[...].astype(F32)
    mem[pl.ds(0, M), :] = m0
    mem[pl.ds(M, M), :] = m0
    with jax.named_scope("xwait"):
      xh.wait()
    for c in qkv_copies(1):
        c.start()
    wo_copy(0).start()
    b_copy(0, 0).start()
    upre = _ln(x0[pl.ds(0, RPRE), :].astype(F32)).astype(BF16)
    lp[...] = upre

    def pre_body(p, c):
        for cp in qkv_copies(p):
            cp.wait()

        @pl.when(p + 2 < NPAIR)
        def _():
            for cp in qkv_copies(p + 2):
                cp.start()

        @pl.when(p + 1 < NPAIR)
        def _():
            wo_copy(p + 1).start()
        for j in range(4):
            @pl.when((p + 1 < NPAIR) & ((p + 1) // 4 == j))
            def _():
                b_copy(j, (p + 1) % 4).start()
        r = pl.ds(pl.multiple_of(p * PW, 128), PW)
        w = jnp.concatenate([wtq[r, :], wtk[r, :], wtv[r, :]], axis=0)
        wt = w.T
        for c_ in range(QW // 128):
            wn[p, c_, :, :] = wt[:, c_ * 128:(c_ + 1) * 128]
        y = jax.lax.dot_general(lp[...], w, NT, preferred_element_type=F32)
        pre[p, pl.ds(0, RPRE), :] = y.astype(BF16)
        return c

    with jax.named_scope("prephase"):
        jax.lax.fori_loop(0, NPAIR, pre_body, 0, unroll=PUNROLL)
    with jax.named_scope("dmawait"):
        xt.start()
        woc.wait()
        for c in bcs:
            c.wait()

    def rows(slot):
        return pl.ds(pl.multiple_of(slot * SEG, SEG), SEG)

    def valid(s):
        return (s >= 0) & (s < NSEG)

    def rslot(s):
        return jnp.where(valid(s), s & (RING - 1), ZSLOT)

    def wslot(s):
        return jnp.where(valid(s), s & (RING - 1), TSLOT)

    def shift_mix(win):
        lane = jax.lax.broadcasted_iota(jnp.int32, (SEG, 128), 1)

        def sh(tile, off):
            return win[HALO + off:HALO + off + SEG, tile * 128:(tile + 1) * 128]
        t0 = sh(0, -1)
        t1 = jnp.where(lane < 32, sh(1, -1), sh(1, 1))
        t2 = jnp.where(lane < 64, sh(2, 1), sh(2, -2))
        t3 = jnp.where(lane < 96, sh(3, -2), sh(3, 2))
        t4 = sh(4, 2)
        return jnp.concatenate([t0, t1, t2, t3, t4], axis=1)

    def ub_load(i):
        return jnp.concatenate([ub[c, pl.ds(i * SEG, SEG), :] for c in range(DT)], axis=1)

    def ub_store(i, val, stores):
        v = val.astype(BF16)
        for c in range(DT):
            stores.append((ub, (c, pl.ds(i * SEG, SEG)), v[:, c * 128:(c + 1) * 128]))

    def a_stage(t, a1, a2, stores):
        res, toks = [], []
        if a1:
            res.append(x0[rows(t), :].astype(F32))
            if a1 in ("now", "ahead"):
                toks.append(ub_load(0))
                nxt = jnp.minimum(t + 1, NSEG - 1) if a1 == "now" else jnp.minimum(
                    t + 1 + NPRE - LAG, NPRE - 1)
                ub_store(0, _ln(x0[rows(nxt), :].astype(F32)), stores)
        if a2:
            res.append(x2[rows(rslot(t - LAG)), :])
            toks.append(ub_load(1))
        if a1 and a2:
            h = jnp.concatenate([mem[...].astype(BF16)] + toks, axis=0)
            m1, m2, t1 = 0, M, 2 * M
            t2 = t1 + (SEG if a1 == "now" else 0)
        else:
            h = jnp.concatenate([mem[pl.ds(0 if a1 else M, M), :], toks[0].astype(F32)], axis=0)
            m1 = m2 = 0
            t1 = t2 = M
        n = len(res)
        acc = None
        y, s, pr, o = {}, {}, {}, {}
        d1, d2, d3, d4 = PIPE

        if a1 == "ahead":
            pview = pre.at[:, pl.ds(pl.multiple_of(t * SEG, SEG), (NPRE - LAG + 1) * SEG), :]

        def qkv(p, j):
            out = []
            c0, c1 = j * PW, (j + 1) * PW
            if a1 == "now":
                out.append(jnp.concatenate([y[p][m1:m1 + M, c0:c1], y[p][t1:t1 + SEG, c0:c1]], axis=0))
            elif a1:
                if a1 == "ahead":
                    tok = pview[p, pl.ds(0, SEG), pl.ds(c0, PW)].astype(F32)
                else:
                    tok = pre[p, rows(t), pl.ds(c0, PW)].astype(F32)
                out.append(jnp.concatenate([y[p][m1:m1 + M, c0:c1], tok], axis=0))
            if a2:
                out.append(jnp.concatenate([y[p][m2:m2 + M, c0:c1], y[p][t2:t2 + SEG, c0:c1]], axis=0))
            return out

        def due(st, j):
            out = []
            for p in range(NPAIR):
                extra = EARLY if p < NEARLY else 0
                extra += LATE[st] if p >= NPAIR - NLATE else 0
                if p + PIPE[st - 1] + extra == j:
                    out.append(p)
            return out

        for j in range(NPAIR + d4 + max(LATE)):
            for st in ORDER:
                if st == 0 and j < NPAIR:
                    y[j] = jnp.dot(h, jnp.concatenate([wn[j, c] for c in range(QW // 128)], axis=1),
                                   preferred_element_type=F32)
                    if a1 == "ahead":
                        pview[j, pl.ds((NPRE - LAG) * SEG, SEG), :] = y[j][t1:t1 + SEG].astype(BF16)
                if st == 1:
                    for p in due(1, j):
                        s[p] = [_scores(q, k) for q, k in zip(qkv(p, 0), qkv(p, 1))]
                if st == 2:
                    for p in due(2, j):
                        pr[p] = [_softmax(a) for a in s.pop(p)]
                if st == 3:
                    for p in due(3, j):
                        o[p] = _cat([_pv(a, v) for a, v in zip(pr.pop(p), qkv(p, 2))])
                        y.pop(p)
                if st == 4:
                    for p in due(4, j):
                        d = jnp.dot(_lhs(o.pop(p)), wo[pl.ds(p * PW, PW), :],
                                    preferred_element_type=F32)
                        acc = d if acc is None else acc + d
            yield
        outs = []
        for i in range(n):
            outs.append((acc[i * L:i * L + M], res[i] + acc[i * L + M:(i + 1) * L]))
        if a1:
            stores.append((mem, (pl.ds(0, M),), outs[0][0]))
            stores.append((x1, (rows(t & (RING - 1)),), outs[0][1]))
        if a2:
            stores.append((mem, (pl.ds(M, M),), outs[-1][0]))
            stores.append((x3, (rows((t - LAG) & (RING - 1)),), outs[-1][1]))

    def bb_chain(sh, zz, xres):
        g = jnp.dot(_lhs(_cat(sh)), w2[...], preferred_element_type=F32)
        yield
        y1 = _cat(zz) + g
        g = jnp.dot(_lhs(_ln(y1)), w3[...], preferred_element_type=F32)
        yield
        g = jnp.dot(_lhs(_gelu(g)), w4[...], preferred_element_type=F32)
        yield
        yield _cat(xres) + (y1 + g)

    def prev_tail(href, s):
        return href[pl.ds(pl.multiple_of(rslot(s - 1) * SEG + SEG - HALO, HALO), HALO), :]

    def b_stage(t, b1, b2, stores):
        lay = []
        if b1:
            lay.append((x1, z1, h1, t - 1, x2))
        if b2:
            lay.append((x3, z2, h2, t - 1 - LAG, None))
        if not lay:
            return
        xin = _cat([l[0][rows(rslot(l[3])), :] for l in lay])
        z = _ln(xin)
        g = jnp.dot(_lhs(_ln(z)), w1[...], preferred_element_type=F32)
        yield
        hh = _gelu(g)
        head = []
        for i, l in enumerate(lay):
            s = l[3]
            hi = jnp.where(valid(s), hh[i * SEG:(i + 1) * SEG], 0.0)
            head.append(hi[0:HALO])
            stores.append((l[1], (rows(wslot(s)),), z[i * SEG:(i + 1) * SEG]))
            stores.append((l[2], (rows(wslot(s)),), hi))
        sh, zz, xres = [], [], []
        for i, l in enumerate(lay):
            s = l[3] - 1
            win = jnp.concatenate([prev_tail(l[2], s), l[2][rows(rslot(s)), :], head[i]], axis=0)
            sh.append(shift_mix(win))
            zz.append(l[1][rows(rslot(s)), :])
            xres.append(l[0][rows(rslot(s)), :])
        chain = bb_chain(sh, zz, xres)
        next(chain)
        yield
        next(chain)
        yield
        next(chain)
        yield
        xn = next(chain)
        for i, l in enumerate(lay):
            s = l[3] - 1
            v = xn[i * SEG:(i + 1) * SEG]
            if l[4] is not None:
                stores.append((l[4], (rows(wslot(s)),), v))
                ub_store(1, _ln(v), stores)
            else:
                so = jnp.where(valid(s), s, NSEG)
                stores.append((obuf, (rows(so),), v.astype(BF16)))

    def step(t, a1, a2, b1, b2, bpos):
        stores = []
        bg = b_stage(t, b1, b2, stores)
        if a1 or a2:
            ag = a_stage(t, a1, a2, stores)
            j = 0
            for _ in ag:
                if j in bpos:
                    next(bg, None)
                j += 1
        for _ in bg:
            pass
        for ref, idx, val in stores:
            ref[idx + (slice(None),)] = val

    def loop(lo, hi, *flags):
        def body(t, c):
            step(t, *flags)
            return c
        with jax.named_scope("loop_%d_%d" % (lo, hi)):
            jax.lax.fori_loop(lo, hi, body, 0)

    T, Fa = True, False

    def prefill(seg):
        st = []
        ub_store(0, _ln(x0[pl.ds(seg * SEG, SEG), :].astype(F32)), st)
        for ref, idx, val in st:
            ref[idx + (slice(None),)] = val

    prefill(NPRE - LAG)
    loop(0, LAG, "ahead", Fa, T, Fa, BPOS0)
    loop(LAG, NPRE, "pre", T, T, T, BPOS1)
    with jax.named_scope("xtwait"):
      xt.wait()
    prefill(NPRE)
    loop(NPRE, NSEG, "now", T, T, T, BPOS2)
    done = NSEG - 5
    oc1 = pltpu.make_async_copy(obuf.at[pl.ds(0, done * SEG), :],
                                out_hbm.at[pl.ds(0, done * SEG), :], osem.at[0])
    oc1.start()
    loop(NSEG, NSEG + LAG, None, T, T, T, BPOS3)

    with jax.named_scope("tail"):
        sa, sb = NSEG - 1, NSEG - 2
        ra, rb, rc = [pl.ds((s % RING) * SEG, SEG) for s in (sa, sb, sb - 1)]
        xa = x3[ra, :]
        za = _ln(xa)
        ha = _gelu(jnp.dot(_lhs(_ln(za)), w1[...], preferred_element_type=F32))
        hb = h2[rb, :]
        winb = jnp.concatenate([h2[rc, :][SEG - HALO:], hb, ha[0:HALO]], axis=0)
        wina = jnp.concatenate([hb[SEG - HALO:], ha, jnp.zeros((HALO, D), F32)], axis=0)
        chain = bb_chain([shift_mix(winb), shift_mix(wina)], [z2[rb, :], za], [x3[rb, :], xa])
        next(chain), next(chain), next(chain)
        obuf[pl.ds(sb * SEG, 2 * SEG), :] = next(chain).astype(BF16)

    with jax.named_scope("outdma"):
        oc2 = pltpu.make_async_copy(obuf.at[pl.ds(done * SEG, S - done * SEG), :],
                                    out_hbm.at[pl.ds(done * SEG, S - done * SEG), :], osem.at[1])
        oc2.start()
        oc1.wait()
        oc2.wait()


@functools.partial(jax.jit, static_argnames=("A_seg_len",))
def pallas_interleave_layers__memory_aug_recurrent_mem_tr__mixer_s_mlp__prompt_kernel(
    A_x, A_mem0, A_Wq, A_Wk, A_Wv, A_Wo, A_seg_len, B_x, B_w1, B_w2, B_w3, B_w4,
):
    del B_x
    assert A_seg_len == SEG and A_x.shape == (1, S, D) and A_mem0.shape == (1, M, D)
    assert A_Wq.shape == (D, H, DH) and A_Wo.shape == (H, DH, D) and B_w3.shape == (D, FF)

    def wt(w):
        return jnp.transpose(w, (1, 2, 0)).reshape(H * DH, D)

    any_spec = pl.BlockSpec(memory_space=pl.ANY)
    out = pl.pallas_call(
        inner_kernel,
        out_shape=jax.ShapeDtypeStruct((S, D), BF16),
        in_specs=[any_spec, pl.BlockSpec(memory_space=pltpu.VMEM)] + [any_spec] * 8,
        out_specs=any_spec,
        scratch_shapes=[
            pltpu.VMEM((H * DH, D), BF16),
            pltpu.VMEM((H * DH, D), BF16),
            pltpu.VMEM((H * DH, D), BF16),
            pltpu.VMEM((NPAIR, QW // 128, D, 128), BF16),
            pltpu.VMEM((H * DH, D), BF16),
            pltpu.VMEM((D, D), BF16),
            pltpu.VMEM((D, D), BF16),
            pltpu.VMEM((D, FF), BF16),
            pltpu.VMEM((FF, D), BF16),
            pltpu.VMEM((S, D), BF16),
            pltpu.VMEM((RPRE, D), BF16),
            pltpu.VMEM((DT, 2 * SEG, 128), BF16),
            pltpu.VMEM((NPAIR, NPRE * SEG, QW), BF16),
            pltpu.VMEM((NSLOT * SEG, D), F32),
            pltpu.VMEM((NSLOT * SEG, D), F32),
            pltpu.VMEM((NSLOT * SEG, D), F32),
            pltpu.VMEM((NSLOT * SEG, D), F32),
            pltpu.VMEM((NSLOT * SEG, D), F32),
            pltpu.VMEM((NSLOT * SEG, D), F32),
            pltpu.VMEM((NSLOT * SEG, D), F32),
            pltpu.VMEM((2 * M, D), F32),
            pltpu.VMEM((S + SEG, D), BF16),
            pltpu.SemaphoreType.DMA((NPAIR,)),
            pltpu.SemaphoreType.DMA((7,)),
            pltpu.SemaphoreType.DMA((2,)),
        ],
        compiler_params=pltpu.CompilerParams(vmem_limit_bytes=120 * 2**20, disable_bounds_checks=True),
    )(A_x.reshape(S, D), A_mem0.reshape(M, D), wt(A_Wq), wt(A_Wk), wt(A_Wv),
      A_Wo.reshape(H * DH, D), B_w1, B_w2, B_w3, B_w4)
    return out.reshape(1, S, D)
```

```python
import functools

import jax
import jax.numpy as jnp
import jax.experimental.pallas as pl
import jax.experimental.pallas.tpu as pltpu

F32 = jnp.float32
BF16 = jnp.bfloat16

S, D, H, DH, M, SEG, FF = 2048, 640, 32, 192, 8, 32, 1536
NSEG = S // SEG
L = M + SEG
NPAIR = H // 2
PW = 2 * DH
QW = 3 * PW
DT = D // 128
LAG = 3
RING = 4
ZSLOT = RING
NSLOT = RING + 1
HALO = 8
EPS = 1e-5
SCALE = DH ** (-0.5)
NT = (((1,), (1,)), ((), ()))
KPRE = 12
NPRE = KPRE + LAG
RPRE = KPRE * SEG
PIPE = (1, 2, 3, 4)
BPOS0 = (4, 8, 12, 16)
BPOS1 = (4, 7, 10, 13)
BPOS2 = (2, 4, 7, 10)
BPOS3 = (10, 13, 15, 17)


def _ln(x):
    m = jnp.mean(x, axis=-1, keepdims=True)
    xc = x - m
    v = jnp.mean(xc * xc, axis=-1, keepdims=True)
    return xc * jax.lax.rsqrt(v + EPS)


def _gelu(x):
    return jax.nn.gelu(x, approximate=True)


def _cat(xs, axis=0):
    return xs[0] if len(xs) == 1 else jnp.concatenate(xs, axis=axis)


def _lhs(x):
    return x.astype(BF16) if x.shape[0] % 16 == 0 else x.astype(F32)


def _mm(a, b):
    return jnp.dot(_lhs(a), b, preferred_element_type=F32)


def _blockdiag(a):
    lane = jax.lax.broadcasted_iota(jnp.int32, (L, 128), 1)
    lo = lane < (DH - 128)
    a0, a1, a2 = a[:, 0:128], a[:, 128:256], a[:, 256:384]
    z = jnp.zeros_like(a0)
    top = jnp.concatenate([a0, jnp.where(lo, a1, 0.0), z], axis=1)
    bot = jnp.concatenate([z, jnp.where(lo, 0.0, a1), a2], axis=1)
    return jnp.concatenate([top, bot], axis=0).astype(BF16)


def _scores(q, k):
    return jax.lax.dot_general(q, _blockdiag(k), NT, preferred_element_type=F32)


def _softmax(s):
    shape = s.shape
    lane = jax.lax.broadcasted_iota(jnp.int32, shape, 1)
    row = jax.lax.broadcasted_iota(jnp.int32, shape, 0) + (L - shape[0])
    h0 = lane < L
    key = jnp.where(h0, lane, lane - L)
    mask = (row < M) | (row >= key)
    s = jnp.where(mask, s * SCALE, -1e9)
    ninf = -jnp.inf
    m0 = jnp.max(jnp.where(h0, s, ninf), axis=-1, keepdims=True)
    m1 = jnp.max(jnp.where(h0, ninf, s), axis=-1, keepdims=True)
    e = jnp.exp(s - jnp.where(h0, m0, m1))
    l0 = jnp.sum(jnp.where(h0, e, 0.0), axis=-1, keepdims=True)
    l1 = jnp.sum(jnp.where(h0, 0.0, e), axis=-1, keepdims=True)
    return e / jnp.where(h0, l0, l1)


def _pv(p, v):
    return jnp.dot(p, _blockdiag(v), preferred_element_type=F32)


def _shift_mix(win):
    lane = jax.lax.broadcasted_iota(jnp.int32, (SEG, 128), 1)

    def sh(tile, off):
        return win[HALO + off:HALO + off + SEG, tile * 128:(tile + 1) * 128]
    c = D // 4
    return jnp.concatenate([
        sh(0, -1),
        jnp.where(lane < c - 128, sh(1, -1), sh(1, 1)),
        jnp.where(lane < 2 * c - 256, sh(2, 1), sh(2, -2)),
        jnp.where(lane < 3 * c - 384, sh(3, -2), sh(3, 2)),
        sh(4, 2)], axis=1)


def _static(t):
    return isinstance(t, int)


def _rows(slot, n=SEG, off=0, unit=SEG):
    if _static(slot):
        return pl.ds(slot * SEG + off, n)
    return pl.ds(pl.multiple_of(slot * SEG + off, unit), n)


def _ring(s):
    return s & (RING - 1)


def inner_kernel(x_hbm, mem0_ref, wq_hbm, wk_hbm, wv_hbm, wo_hbm,
                 w1_hbm, w2_hbm, w3_hbm, w4_hbm,
                 out_hbm,
                 wtq, wtk, wtv, wn, wo, w1, w2, w3, w4,
                 x0, lp, ub, pre, x1, x2, x3, z1, z2, h1, h2, mem, obuf,
                 qsem, sems):

    def blk(i, n, unit):
        return pl.ds(i * n if _static(i) else pl.multiple_of(i * n, unit), n)

    def qkv_copies(p):
        r = blk(p, PW, 128)
        return [pltpu.make_async_copy(a.at[r, :], b.at[r, :], qsem.at[p & 3])
                for a, b in ((wq_hbm, wtq), (wk_hbm, wtk), (wv_hbm, wtv))]

    def wo_copy(p):
        r = blk(p, PW, 128)
        return pltpu.make_async_copy(wo_hbm.at[r, :], wo.at[r, :], sems.at[2])

    bws = ((w1_hbm, w1), (w2_hbm, w2), (w3_hbm, w3), (w4_hbm, w4))

    def b_copy(j, i):
        a, b = bws[j]
        r = blk(i, b.shape[0] // 4, 16)
        return pltpu.make_async_copy(a.at[r, :], b.at[r, :], sems.at[3 + j])

    hd = NPRE * SEG
    xh = pltpu.make_async_copy(x_hbm.at[pl.ds(0, hd), :], x0.at[pl.ds(0, hd), :], sems.at[0])
    xt = pltpu.make_async_copy(x_hbm.at[pl.ds(hd, S - hd), :], x0.at[pl.ds(hd, S - hd), :],
                               sems.at[1])
    xh.start()
    for cp in qkv_copies(0):
        cp.start()

    zero = jnp.zeros((SEG, D), F32)
    for b in (h1, h2):
        b[_rows(ZSLOT), :] = zero
    m0 = mem0_ref[...].astype(F32)
    mem[pl.ds(0, M), :] = m0
    mem[pl.ds(M, M), :] = m0

    xh.wait()
    for cp in qkv_copies(1):
        cp.start()
    wo_copy(0).start()
    b_copy(0, 0).start()
    lp[...] = _ln(x0[pl.ds(0, RPRE), :].astype(F32)).astype(BF16)

    def pre_body(p, c):
        for cp in qkv_copies(p):
            cp.wait()

        @pl.when(p + 2 < NPAIR)
        def _():
            for cp in qkv_copies(p + 2):
                cp.start()

        @pl.when(p + 1 < NPAIR)
        def _():
            wo_copy(p + 1).start()
        for j in range(4):
            @pl.when((p + 1 < NPAIR) & ((p + 1) // 4 == j))
            def _():
                b_copy(j, (p + 1) % 4).start()
        r = blk(p, PW, 128)
        w = jnp.concatenate([wtq[r, :], wtk[r, :], wtv[r, :]], axis=0)
        wt = w.T
        for c_ in range(QW // 128):
            wn[p, c_, :, :] = wt[:, c_ * 128:(c_ + 1) * 128]
        y = jax.lax.dot_general(lp[...], w, NT, preferred_element_type=F32)
        pre[p, pl.ds(0, RPRE), :] = y.astype(BF16)
        return c

    with jax.named_scope("prephase"):
        jax.lax.fori_loop(0, NPAIR, pre_body, 0)
    xt.start()
    pltpu.make_async_copy(wo_hbm, wo, sems.at[2]).wait()
    for j, (a, b) in enumerate(bws):
        pltpu.make_async_copy(a, b, sems.at[3 + j]).wait()

    def ub_load(i):
        return jnp.concatenate([ub[c, pl.ds(i * SEG, SEG), :] for c in range(DT)], axis=1)

    def ub_store(i, val, stores):
        v = val.astype(BF16)
        for c in range(DT):
            stores.append((ub, (c, pl.ds(i * SEG, SEG)), v[:, c * 128:(c + 1) * 128]))

    def wcols(p, lo, hi):
        return jnp.concatenate([wn[p, c] for c in range(lo, hi)], axis=1)

    def a_stage(t, a1, a2, stores):
        last1 = _static(t) and t == NSEG - 1
        last2 = _static(t) and t - LAG == NSEG - 1
        res, toks = [], []
        if a1:
            res.append(x0[_rows(t), :].astype(F32))
            if a1 != "pre":
                toks.append(ub_load(0))
            if a1 == "ahead" and t + 1 < LAG:
                ub_store(0, _ln(x0[_rows(t + 1 + KPRE), :].astype(F32)), stores)
            if a1 == "now" and not last1:
                ub_store(0, _ln(x0[_rows(t + 1), :].astype(F32)), stores)
        if a2:
            res.append(x2[_rows(_ring(t - LAG)), :])
            toks.append(ub_load(1))
        if a1 and a2:
            h = jnp.concatenate([mem[...].astype(BF16)] + toks, axis=0)
            m1, m2, t1 = 0, M, 2 * M
            t2 = t1 + (SEG if a1 == "now" else 0)
        else:
            h = jnp.concatenate([mem[pl.ds(0 if a1 else M, M), :], toks[0].astype(F32)], axis=0)
            m1 = m2 = 0
            t1 = t2 = M
        hq = _lhs(h[M:]) if (last1 or last2) else None

        def project(p):
            if hq is None:
                y = jnp.dot(h, wcols(p, 0, 9), preferred_element_type=F32)
                return y[:, 0:PW], y[:, PW:2 * PW], y[:, 2 * PW:]
            yq = jnp.dot(hq, wcols(p, 0, 3), preferred_element_type=F32)
            y = jnp.dot(h, wcols(p, 3, 9), preferred_element_type=F32)
            return yq, y[:, 0:PW], y[:, PW:]

        def split(yj, p, j):
            qo = M if (j == 0 and hq is not None) else 0
            out = []
            if a1:
                if a1 == "now":
                    tok = yj[t1 - qo:t1 - qo + SEG]
                else:
                    tok = pre[p, _rows(t), pl.ds(j * PW, PW)].astype(F32)
                out.append(tok if (j == 0 and last1)
                           else jnp.concatenate([yj[m1:m1 + M], tok], axis=0))
            if a2:
                tok = yj[t2 - qo:t2 - qo + SEG]
                out.append(tok if (j == 0 and last2)
                           else jnp.concatenate([yj[m2 - qo:m2 - qo + M], tok], axis=0))
            return out

        acc = None
        y, s, pr, o = {}, {}, {}, {}
        d1, d2, d3, d4 = PIPE
        for j in range(NPAIR + d4):
            if j < NPAIR:
                y[j] = project(j)
                if a1 == "ahead":
                    pre[j, _rows(t + KPRE), :] = jnp.concatenate(
                        [a[t1:t1 + SEG] for a in y[j]], axis=1).astype(BF16)
            p = j - d1
            if 0 <= p < NPAIR:
                s[p] = [_scores(q, k) for q, k in zip(split(y[p][0], p, 0), split(y[p][1], p, 1))]
            p = j - d2
            if 0 <= p < NPAIR:
                pr[p] = [_softmax(a) for a in s.pop(p)]
            p = j - d3
            if 0 <= p < NPAIR:
                o[p] = _cat([_pv(a, v) for a, v in zip(pr.pop(p), split(y.pop(p)[2], p, 2))])
            p = j - d4
            if 0 <= p < NPAIR:
                d = _mm(o.pop(p), wo[pl.ds(p * PW, PW), :])
                acc = d if acc is None else acc + d
            yield
        r = 0
        if a1:
            if not last1:
                stores.append((mem, (pl.ds(0, M),), acc[0:M]))
                r = M
            stores.append((x1, (_rows(_ring(t)),), res[0] + acc[r:r + SEG]))
            r += SEG
        if a2:
            if not last2:
                stores.append((mem, (pl.ds(M, M),), acc[r:r + M]))
                r += M
            stores.append((x3, (_rows(_ring(t - LAG)),), res[-1] + acc[r:r + SEG]))

    def bb_chain(sh, zz, xres):
        g = _mm(_cat(sh), w2[...])
        yield
        y1 = _cat(zz) + g
        g = _mm(_ln(y1), w3[...])
        yield
        g = _mm(_gelu(g), w4[...])
        yield
        yield _cat(xres) + (y1 + g)

    def prev_tail(href, s):
        if _static(s):
            slot = ZSLOT if s == 0 else _ring(s - 1)
        else:
            slot = jnp.where(s == 0, ZSLOT, _ring(s - 1))
        return href[_rows(slot, HALO, SEG - HALO, HALO), :]

    def b_stage(t, b1, b2, stores):
        lay = [(x1, z1, h1, t - 1, x2, b1), (x3, z2, h2, t - 1 - LAG, None, b2)]
        ba = [i for i, l in enumerate(lay) if l[5][0]]
        bb = [i for i, l in enumerate(lay) if l[5][1]]
        head = {}
        if ba:
            z = _ln(_cat([lay[i][0][_rows(_ring(lay[i][3])), :] for i in ba]))
            g = _mm(_ln(z), w1[...])
        yield
        if ba:
            hh = _gelu(g)
            for n, i in enumerate(ba):
                _, zr, hr, s, _, _ = lay[i]
                hi = hh[n * SEG:(n + 1) * SEG]
                head[i] = hi[0:HALO]
                stores.append((zr, (_rows(_ring(s)),), z[n * SEG:(n + 1) * SEG]))
                stores.append((hr, (_rows(_ring(s)),), hi))
        if not bb:
            return
        sh, zz, xres = [], [], []
        for i in bb:
            xr, zr, hr, s, _, _ = lay[i]
            s = s - 1
            nxt = head[i] if i in head else jnp.zeros((HALO, D), F32)
            sh.append(_shift_mix(jnp.concatenate(
                [prev_tail(hr, s), hr[_rows(_ring(s)), :], nxt], axis=0)))
            zz.append(zr[_rows(_ring(s)), :])
            xres.append(xr[_rows(_ring(s)), :])
        chain = bb_chain(sh, zz, xres)
        for _ in range(3):
            next(chain)
            yield
        xn = next(chain)
        for n, i in enumerate(bb):
            s = lay[i][3] - 1
            v = xn[n * SEG:(n + 1) * SEG]
            if lay[i][4] is not None:
                stores.append((lay[i][4], (_rows(_ring(s)),), v))
                ub_store(1, _ln(v), stores)
            else:
                stores.append((obuf, (_rows(s),), v.astype(BF16)))

    def step(t, a1, a2, b1, b2, bpos):
        stores = []
        bg = b_stage(t, b1, b2, stores)
        for j, _ in enumerate(a_stage(t, a1, a2, stores)):
            if j in bpos:
                next(bg, None)
        for _ in bg:
            pass
        for ref, idx, val in stores:
            ref[idx + (slice(None),)] = val

    def auto(t, a1, bpos):
        ok = lambda s: 0 <= s < NSEG
        step(t, a1 if ok(t) else None, ok(t - LAG),
             (ok(t - 1), ok(t - 2)), (ok(t - 1 - LAG), ok(t - 2 - LAG)), bpos)

    def loop(lo, hi, a1, bpos):
        def body(t, c):
            step(t, a1, True, (True, True), (True, True), bpos)
            return c
        with jax.named_scope("loop_%d_%d" % (lo, hi)):
            jax.lax.fori_loop(lo, hi, body, 0)

    def prefill(seg):
        st = []
        ub_store(0, _ln(x0[_rows(seg), :].astype(F32)), st)
        for ref, idx, val in st:
            ref[idx + (slice(None),)] = val

    def out_copy(lo, hi, i):
        r = pl.ds(lo * SEG, (hi - lo) * SEG)
        return pltpu.make_async_copy(obuf.at[r, :], out_hbm.at[r, :], sems.at[i])

    prefill(KPRE)
    with jax.named_scope("steps_v0"):
        for t in range(LAG):
            auto(t, "ahead", BPOS0)
    with jax.named_scope("steps_v1"):
        for t in range(LAG, LAG + 2):
            auto(t, "pre", BPOS1)
    loop(LAG + 2, NPRE, "pre", BPOS1)
    xt.wait()
    prefill(NPRE)
    loop(NPRE, NSEG - 1, "now", BPOS2)
    with jax.named_scope("steps_v2"):
        auto(NSEG - 1, "now", BPOS2)
    done = NSEG - 5
    out_copy(0, done, 0).start()
    with jax.named_scope("steps_v3"):
        for t in range(NSEG, NSEG + LAG):
            auto(t, None, BPOS3)

    with jax.named_scope("tail"):
        sa, sb = NSEG - 1, NSEG - 2
        xa, xb = x3[_rows(_ring(sa)), :], x3[_rows(_ring(sb)), :]
        za = _ln(xa)
        ha = _gelu(_mm(_ln(za), w1[...]))
        hb = h2[_rows(_ring(sb)), :]
        winb = jnp.concatenate([prev_tail(h2, sb), hb, ha[0:HALO]], axis=0)
        wina = jnp.concatenate([hb[SEG - HALO:], ha, jnp.zeros((HALO, D), F32)], axis=0)
        chain = bb_chain([_shift_mix(winb), _shift_mix(wina)], [z2[_rows(_ring(sb)), :], za], [xb, xa])
        for _ in range(3):
            next(chain)
        obuf[pl.ds(sb * SEG, 2 * SEG), :] = next(chain).astype(BF16)

    out_copy(done, NSEG, 1).start()
    out_copy(0, done, 0).wait()
    out_copy(done, NSEG, 1).wait()


@functools.partial(jax.jit, static_argnames=("A_seg_len",))
def pallas_interleave_layers__memory_aug_recurrent_mem_tr__mixer_s_mlp__prompt_kernel(
    A_x, A_mem0, A_Wq, A_Wk, A_Wv, A_Wo, A_seg_len, B_x, B_w1, B_w2, B_w3, B_w4,
):
    del B_x
    assert A_seg_len == SEG and A_x.shape == (1, S, D) and A_mem0.shape == (1, M, D)
    assert A_Wq.shape == (D, H, DH) and A_Wo.shape == (H, DH, D) and B_w3.shape == (D, FF)

    def wt(w):
        return jnp.transpose(w, (1, 2, 0)).reshape(H * DH, D)

    any_spec = pl.BlockSpec(memory_space=pl.ANY)
    ring = pltpu.VMEM((RING * SEG, D), F32)
    out = pl.pallas_call(
        inner_kernel,
        out_shape=jax.ShapeDtypeStruct((S, D), BF16),
        in_specs=[any_spec, pl.BlockSpec(memory_space=pltpu.VMEM)] + [any_spec] * 8,
        out_specs=any_spec,
        scratch_shapes=[
            pltpu.VMEM((H * DH, D), BF16),
            pltpu.VMEM((H * DH, D), BF16),
            pltpu.VMEM((H * DH, D), BF16),
            pltpu.VMEM((NPAIR, QW // 128, D, 128), BF16),
            pltpu.VMEM((H * DH, D), BF16),
            pltpu.VMEM((D, D), BF16),
            pltpu.VMEM((D, D), BF16),
            pltpu.VMEM((D, FF), BF16),
            pltpu.VMEM((FF, D), BF16),
            pltpu.VMEM((S, D), BF16),
            pltpu.VMEM((RPRE, D), BF16),
            pltpu.VMEM((DT, 2 * SEG, 128), BF16),
            pltpu.VMEM((NPAIR, NPRE * SEG, QW), BF16),
            ring, ring, ring,
            ring, ring,
            pltpu.VMEM((NSLOT * SEG, D), F32),
            pltpu.VMEM((NSLOT * SEG, D), F32),
            pltpu.VMEM((2 * M, D), F32),
            pltpu.VMEM((S, D), BF16),
            pltpu.SemaphoreType.DMA((4,)),
            pltpu.SemaphoreType.DMA((7,)),
        ],
        compiler_params=pltpu.CompilerParams(vmem_limit_bytes=120 * 2**20,
                                             disable_bounds_checks=True),
    )(A_x.reshape(S, D), A_mem0.reshape(M, D), wt(A_Wq), wt(A_Wk), wt(A_Wv),
      A_Wo.reshape(H * DH, D), B_w1, B_w2, B_w3, B_w4)
    return out.reshape(1, S, D)
```

```python
import functools

import jax
import jax.numpy as jnp
import jax.experimental.pallas as pl
import jax.experimental.pallas.tpu as pltpu

F32 = jnp.float32
BF16 = jnp.bfloat16

S, D, H, DH, M, SEG, FF = 2048, 640, 32, 192, 8, 32, 1536
NSEG = S // SEG
L = M + SEG
NPAIR = H // 2
PW = 2 * DH
QW = 3 * PW
DT = D // 128
LAG = 3
RING = 4
ZSLOT = RING
NSLOT = RING + 1
HALO = 8
EPS = 1e-5
SCALE = DH ** (-0.5)
NT = (((1,), (1,)), ((), ()))
KPRE = 12
NPRE = KPRE + LAG
RPRE = KPRE * SEG
PIPE = (1, 2, 3, 4)
BPOS_HEAD, BPOS_PRE, BPOS_MAIN, BPOS_LAST, BPOS_TAIL = (
    (4, 8, 12, 16), (4, 6, 8, 10), (2, 4, 6, 8), (2, 4, 7, 10), (10, 13, 15, 17))


def _ln(x):
    m = jnp.mean(x, axis=-1, keepdims=True)
    xc = x - m
    v = jnp.mean(xc * xc, axis=-1, keepdims=True)
    return xc * jax.lax.rsqrt(v + EPS)


def _gelu(x):
    return jax.nn.gelu(x, approximate=True)


def _cat(xs, axis=0):
    return xs[0] if len(xs) == 1 else jnp.concatenate(xs, axis=axis)


def _lhs(x):
    return x.astype(BF16) if x.shape[0] % 16 == 0 else x.astype(F32)


def _mm(a, b):
    return jnp.dot(_lhs(a), b, preferred_element_type=F32)


def _blockdiag(a):
    lane = jax.lax.broadcasted_iota(jnp.int32, (L, 128), 1)
    lo = lane < (DH - 128)
    a0, a1, a2 = a[:, 0:128], a[:, 128:256], a[:, 256:384]
    z = jnp.zeros_like(a0)
    top = jnp.concatenate([a0, jnp.where(lo, a1, 0.0), z], axis=1)
    bot = jnp.concatenate([z, jnp.where(lo, 0.0, a1), a2], axis=1)
    return jnp.concatenate([top, bot], axis=0).astype(BF16)


def _scores(q, k):
    return jax.lax.dot_general(q, _blockdiag(k), NT, preferred_element_type=F32)


def _softmax(s):
    shape = s.shape
    lane = jax.lax.broadcasted_iota(jnp.int32, shape, 1)
    row = jax.lax.broadcasted_iota(jnp.int32, shape, 0) + (L - shape[0])
    h0 = lane < L
    key = jnp.where(h0, lane, lane - L)
    mask = (row < M) | (row >= key)
    s = jnp.where(mask, s * SCALE, -1e9)
    ninf = -jnp.inf
    m0 = jnp.max(jnp.where(h0, s, ninf), axis=-1, keepdims=True)
    m1 = jnp.max(jnp.where(h0, ninf, s), axis=-1, keepdims=True)
    e = jnp.exp(s - jnp.where(h0, m0, m1))
    l0 = jnp.sum(jnp.where(h0, e, 0.0), axis=-1, keepdims=True)
    l1 = jnp.sum(jnp.where(h0, 0.0, e), axis=-1, keepdims=True)
    return e / jnp.where(h0, l0, l1)


def _pv(p, v):
    return jnp.dot(p, _blockdiag(v), preferred_element_type=F32)


def _shift_mix(win):
    lane = jax.lax.broadcasted_iota(jnp.int32, (SEG, 128), 1)

    def sh(tile, off):
        return win[HALO + off:HALO + off + SEG, tile * 128:(tile + 1) * 128]
    c = D // 4
    return jnp.concatenate([
        sh(0, -1),
        jnp.where(lane < c - 128, sh(1, -1), sh(1, 1)),
        jnp.where(lane < 2 * c - 256, sh(2, 1), sh(2, -2)),
        jnp.where(lane < 3 * c - 384, sh(3, -2), sh(3, 2)),
        sh(4, 2)], axis=1)


def _static(t):
    return isinstance(t, int)


def _rows(slot, n=SEG, off=0, unit=SEG):
    if _static(slot):
        return pl.ds(slot * SEG + off, n)
    return pl.ds(pl.multiple_of(slot * SEG + off, unit), n)


def _ring(s):
    return s & (RING - 1)


def inner_kernel(x_hbm, mem0_ref, wq_hbm, wk_hbm, wv_hbm, wo_hbm,
                 w1_hbm, w2_hbm, w3_hbm, w4_hbm,
                 out_hbm,
                 wtq, wtk, wtv, wn, wo, w1, w2, w3, w4,
                 x0, lp, ub, pre, x1, x2, x3, z1, z2, h1, h2, mem, obuf,
                 qsem, sems):

    def blk(i, n, unit):
        return pl.ds(i * n if _static(i) else pl.multiple_of(i * n, unit), n)

    def qkv_copies(p):
        r = blk(p, PW, 128)
        return [pltpu.make_async_copy(a.at[r, :], b.at[r, :], qsem.at[p & 3])
                for a, b in ((wq_hbm, wtq), (wk_hbm, wtk), (wv_hbm, wtv))]

    def wo_copy(p):
        r = blk(p, PW, 128)
        return pltpu.make_async_copy(wo_hbm.at[r, :], wo.at[r, :], sems.at[2])

    bws = ((w1_hbm, w1), (w2_hbm, w2), (w3_hbm, w3), (w4_hbm, w4))

    def b_copy(j, i):
        a, b = bws[j]
        r = blk(i, b.shape[0] // 4, 16)
        return pltpu.make_async_copy(a.at[r, :], b.at[r, :], sems.at[3 + j])

    hd = NPRE * SEG
    xh = pltpu.make_async_copy(x_hbm.at[pl.ds(0, hd), :], x0.at[pl.ds(0, hd), :], sems.at[0])
    xt = pltpu.make_async_copy(x_hbm.at[pl.ds(hd, S - hd), :], x0.at[pl.ds(hd, S - hd), :],
                               sems.at[1])
    xh.start()
    for cp in qkv_copies(0):
        cp.start()

    zero = jnp.zeros((SEG, D), F32)
    for b in (h1, h2):
        b[_rows(ZSLOT), :] = zero
    m0 = mem0_ref[...].astype(F32)
    mem[pl.ds(0, M), :] = m0
    mem[pl.ds(M, M), :] = m0

    xh.wait()
    for cp in qkv_copies(1):
        cp.start()
    wo_copy(0).start()
    b_copy(0, 0).start()
    lp[...] = _ln(x0[pl.ds(0, RPRE), :].astype(F32)).astype(BF16)

    def pre_body(p, c):
        for cp in qkv_copies(p):
            cp.wait()

        @pl.when(p + 2 < NPAIR)
        def _():
            for cp in qkv_copies(p + 2):
                cp.start()

        @pl.when(p + 1 < NPAIR)
        def _():
            wo_copy(p + 1).start()
        for j in range(4):
            @pl.when((p + 1 < NPAIR) & ((p + 1) // 4 == j))
            def _():
                b_copy(j, (p + 1) % 4).start()
        r = blk(p, PW, 128)
        w = jnp.concatenate([wtq[r, :], wtk[r, :], wtv[r, :]], axis=0)
        wt = w.T
        for c_ in range(QW // 128):
            wn[p, c_, :, :] = wt[:, c_ * 128:(c_ + 1) * 128]
        y = jax.lax.dot_general(lp[...], w, NT, preferred_element_type=F32)
        pre[p, pl.ds(0, RPRE), :] = y.astype(BF16)
        return c

    jax.lax.fori_loop(0, NPAIR, pre_body, 0)
    xt.start()
    pltpu.make_async_copy(wo_hbm, wo, sems.at[2]).wait()
    for j, (a, b) in enumerate(bws):
        pltpu.make_async_copy(a, b, sems.at[3 + j]).wait()

    def ub_load(i):
        return jnp.concatenate([ub[c, pl.ds(i * SEG, SEG), :] for c in range(DT)], axis=1)

    def ub_store(i, val, stores):
        v = val.astype(BF16)
        for c in range(DT):
            stores.append((ub, (c, pl.ds(i * SEG, SEG)), v[:, c * 128:(c + 1) * 128]))

    def wcols(p, lo, hi):
        return jnp.concatenate([wn[p, c] for c in range(lo, hi)], axis=1)

    def a_stage(t, a1, a2, stores):
        last1 = _static(t) and t == NSEG - 1
        last2 = _static(t) and t - LAG == NSEG - 1
        res, toks = [], []
        if a1:
            res.append(x0[_rows(t), :].astype(F32))
            if a1 != "pre":
                toks.append(ub_load(0))
            if a1 == "ahead" and t + 1 < LAG:
                ub_store(0, _ln(x0[_rows(t + 1 + KPRE), :].astype(F32)), stores)
            if a1 == "now" and not last1:
                ub_store(0, _ln(x0[_rows(t + 1), :].astype(F32)), stores)
        if a2:
            res.append(x2[_rows(_ring(t - LAG)), :])
            toks.append(ub_load(1))
        if a1 and a2:
            h = jnp.concatenate([mem[...].astype(BF16)] + toks, axis=0)
            m1, m2, t1 = 0, M, 2 * M
            t2 = t1 + (SEG if a1 == "now" else 0)
        else:
            h = jnp.concatenate([mem[pl.ds(0 if a1 else M, M), :], toks[0].astype(F32)], axis=0)
            m1 = m2 = 0
            t1 = t2 = M
        hq = _lhs(h[M:]) if (last1 or last2) else None

        def project(p):
            if hq is None:
                y = jnp.dot(h, wcols(p, 0, 9), preferred_element_type=F32)
                return y[:, 0:PW], y[:, PW:2 * PW], y[:, 2 * PW:]
            yq = jnp.dot(hq, wcols(p, 0, 3), preferred_element_type=F32)
            y = jnp.dot(h, wcols(p, 3, 9), preferred_element_type=F32)
            return yq, y[:, 0:PW], y[:, PW:]

        def split(yj, p, j):
            qo = M if (j == 0 and hq is not None) else 0
            out = []
            if a1:
                if a1 == "now":
                    tok = yj[t1 - qo:t1 - qo + SEG]
                else:
                    tok = pre[p, _rows(t), pl.ds(j * PW, PW)].astype(F32)
                out.append(tok if (j == 0 and last1)
                           else jnp.concatenate([yj[m1:m1 + M], tok], axis=0))
            if a2:
                tok = yj[t2 - qo:t2 - qo + SEG]
                out.append(tok if (j == 0 and last2)
                           else jnp.concatenate([yj[m2 - qo:m2 - qo + M], tok], axis=0))
            return out

        acc = None
        y, s, pr, o = {}, {}, {}, {}
        d1, d2, d3, d4 = PIPE
        for j in range(NPAIR + d4):
            if j < NPAIR:
                y[j] = project(j)
                if a1 == "ahead":
                    pre[j, _rows(t + KPRE), :] = jnp.concatenate(
                        [a[t1:t1 + SEG] for a in y[j]], axis=1).astype(BF16)
            p = j - d1
            if 0 <= p < NPAIR:
                s[p] = [_scores(q, k) for q, k in zip(split(y[p][0], p, 0), split(y[p][1], p, 1))]
            p = j - d2
            if 0 <= p < NPAIR:
                pr[p] = [_softmax(a) for a in s.pop(p)]
            p = j - d3
            if 0 <= p < NPAIR:
                o[p] = _cat([_pv(a, v) for a, v in zip(pr.pop(p), split(y.pop(p)[2], p, 2))])
            p = j - d4
            if 0 <= p < NPAIR:
                d = _mm(o.pop(p), wo[pl.ds(p * PW, PW), :])
                acc = d if acc is None else acc + d
            yield
        r = 0
        if a1:
            if not last1:
                stores.append((mem, (pl.ds(0, M),), acc[0:M]))
                r = M
            stores.append((x1, (_rows(_ring(t)),), res[0] + acc[r:r + SEG]))
            r += SEG
        if a2:
            if not last2:
                stores.append((mem, (pl.ds(M, M),), acc[r:r + M]))
                r += M
            stores.append((x3, (_rows(_ring(t - LAG)),), res[-1] + acc[r:r + SEG]))

    def bb_chain(sh, zz, xres):
        g = _mm(_cat(sh), w2[...])
        yield
        y1 = _cat(zz) + g
        g = _mm(_ln(y1), w3[...])
        yield
        g = _mm(_gelu(g), w4[...])
        yield
        yield _cat(xres) + (y1 + g)

    def prev_tail(href, s):
        if _static(s):
            slot = ZSLOT if s == 0 else _ring(s - 1)
        else:
            slot = jnp.where(s == 0, ZSLOT, _ring(s - 1))
        return href[_rows(slot, HALO, SEG - HALO, HALO), :]

    def b_stage(t, b1, b2, stores):
        lay = [(x1, z1, h1, t - 1, x2, b1), (x3, z2, h2, t - 1 - LAG, None, b2)]
        ba = [i for i, l in enumerate(lay) if l[5][0]]
        bb = [i for i, l in enumerate(lay) if l[5][1]]
        head = {}
        zv = {}
        for i in set(ba) & set(bb):
            if not _static(t):
                zv[i] = lay[i][1].at[_rows(lay[i][3] - 1, 2 * SEG), :]
        if ba:
            z = _ln(_cat([lay[i][0][_rows(_ring(lay[i][3])), :] for i in ba]))
            g = _mm(_ln(z), w1[...])
        yield
        if ba:
            hh = _gelu(g)
            for n, i in enumerate(ba):
                _, zr, hr, s, _, _ = lay[i]
                hi = hh[n * SEG:(n + 1) * SEG]
                head[i] = hi[0:HALO]
                if i in zv:
                    zv[i][pl.ds(SEG, SEG), :] = z[n * SEG:(n + 1) * SEG]
                else:
                    zr[_rows(s), :] = z[n * SEG:(n + 1) * SEG]
                stores.append((hr, (_rows(_ring(s)),), hi))
        if not bb:
            return
        sh, zz, xres = [], [], []
        for i in bb:
            xr, zr, hr, s, _, _ = lay[i]
            s = s - 1
            nxt = head[i] if i in head else jnp.zeros((HALO, D), F32)
            sh.append(_shift_mix(jnp.concatenate(
                [prev_tail(hr, s), hr[_rows(_ring(s)), :], nxt], axis=0)))
            zz.append(zv[i][pl.ds(0, SEG), :] if i in zv else zr[_rows(s), :])
            xres.append(xr[_rows(_ring(s)), :])
        chain = bb_chain(sh, zz, xres)
        for _ in range(3):
            next(chain)
            yield
        xn = next(chain)
        for n, i in enumerate(bb):
            s = lay[i][3] - 1
            v = xn[n * SEG:(n + 1) * SEG]
            if lay[i][4] is not None:
                stores.append((lay[i][4], (_rows(_ring(s)),), v))
                ub_store(1, _ln(v), stores)
            else:
                stores.append((obuf, (_rows(s),), v.astype(BF16)))

    def step(t, a1, a2, b1, b2, bpos):
        stores = []
        bg = b_stage(t, b1, b2, stores)
        for j, _ in enumerate(a_stage(t, a1, a2, stores)):
            if j in bpos:
                next(bg, None)
        for _ in bg:
            pass
        for ref, idx, val in stores:
            ref[idx + (slice(None),)] = val

    def auto(t, a1, bpos):
        ok = lambda s: 0 <= s < NSEG
        step(t, a1 if ok(t) else None, ok(t - LAG),
             (ok(t - 1), ok(t - 2)), (ok(t - 1 - LAG), ok(t - 2 - LAG)), bpos)

    def loop(lo, hi, a1, bpos):
        def body(t, c):
            step(t, a1, True, (True, True), (True, True), bpos)
            return c
        jax.lax.fori_loop(lo, hi, body, 0)

    def prefill(seg):
        st = []
        ub_store(0, _ln(x0[_rows(seg), :].astype(F32)), st)
        for ref, idx, val in st:
            ref[idx + (slice(None),)] = val

    def out_copy(lo, hi, i):
        r = pl.ds(lo * SEG, (hi - lo) * SEG)
        return pltpu.make_async_copy(obuf.at[r, :], out_hbm.at[r, :], sems.at[i])

    prefill(KPRE)
    for t in range(LAG):
        auto(t, "ahead", BPOS_HEAD)
    for t in range(LAG, LAG + 2):
        auto(t, "pre", BPOS_PRE)
    loop(LAG + 2, NPRE, "pre", BPOS_PRE)
    xt.wait()
    prefill(NPRE)
    loop(NPRE, NSEG - 1, "now", BPOS_MAIN)
    auto(NSEG - 1, "now", BPOS_LAST)
    done = NSEG - 5
    out_copy(0, done, 0).start()
    for t in range(NSEG, NSEG + LAG):
        auto(t, None, BPOS_TAIL)

    sa, sb = NSEG - 1, NSEG - 2
    xa, xb = x3[_rows(_ring(sa)), :], x3[_rows(_ring(sb)), :]
    za = _ln(xa)
    ha = _gelu(_mm(_ln(za), w1[...]))
    hb = h2[_rows(_ring(sb)), :]
    winb = jnp.concatenate([prev_tail(h2, sb), hb, ha[0:HALO]], axis=0)
    wina = jnp.concatenate([hb[SEG - HALO:], ha, jnp.zeros((HALO, D), F32)], axis=0)
    chain = bb_chain([_shift_mix(winb), _shift_mix(wina)], [z2[_rows(sb), :], za], [xb, xa])
    for _ in range(3):
        next(chain)
    obuf[pl.ds(sb * SEG, 2 * SEG), :] = next(chain).astype(BF16)

    out_copy(done, NSEG, 1).start()
    out_copy(0, done, 0).wait()
    out_copy(done, NSEG, 1).wait()


@functools.partial(jax.jit, static_argnames=("A_seg_len",))
def pallas_interleave_layers__memory_aug_recurrent_mem_tr__mixer_s_mlp__prompt_kernel(
    A_x, A_mem0, A_Wq, A_Wk, A_Wv, A_Wo, A_seg_len, B_x, B_w1, B_w2, B_w3, B_w4,
):
    del B_x
    assert A_seg_len == SEG and A_x.shape == (1, S, D) and A_mem0.shape == (1, M, D)
    assert A_Wq.shape == (D, H, DH) and A_Wo.shape == (H, DH, D) and B_w3.shape == (D, FF)

    def wt(w):
        return jnp.transpose(w, (1, 2, 0)).reshape(H * DH, D)

    any_spec = pl.BlockSpec(memory_space=pl.ANY)
    ring = pltpu.VMEM((RING * SEG, D), F32)
    out = pl.pallas_call(
        inner_kernel,
        out_shape=jax.ShapeDtypeStruct((S, D), BF16),
        in_specs=[any_spec, pl.BlockSpec(memory_space=pltpu.VMEM)] + [any_spec] * 8,
        out_specs=any_spec,
        scratch_shapes=[
            pltpu.VMEM((H * DH, D), BF16),
            pltpu.VMEM((H * DH, D), BF16),
            pltpu.VMEM((H * DH, D), BF16),
            pltpu.VMEM((NPAIR, QW // 128, D, 128), BF16),
            pltpu.VMEM((H * DH, D), BF16),
            pltpu.VMEM((D, D), BF16),
            pltpu.VMEM((D, D), BF16),
            pltpu.VMEM((D, FF), BF16),
            pltpu.VMEM((FF, D), BF16),
            pltpu.VMEM((S, D), BF16),
            pltpu.VMEM((RPRE, D), BF16),
            pltpu.VMEM((DT, 2 * SEG, 128), BF16),
            pltpu.VMEM((NPAIR, NPRE * SEG, QW), BF16),
            ring, ring, ring,
            pltpu.VMEM((S, D), F32), pltpu.VMEM((S, D), F32),
            pltpu.VMEM((NSLOT * SEG, D), F32),
            pltpu.VMEM((NSLOT * SEG, D), F32),
            pltpu.VMEM((2 * M, D), F32),
            pltpu.VMEM((S, D), BF16),
            pltpu.SemaphoreType.DMA((4,)),
            pltpu.SemaphoreType.DMA((7,)),
        ],
        compiler_params=pltpu.CompilerParams(vmem_limit_bytes=120 * 2**20,
                                             disable_bounds_checks=True),
    )(A_x.reshape(S, D), A_mem0.reshape(M, D), wt(A_Wq), wt(A_Wk), wt(A_Wv),
      A_Wo.reshape(H * DH, D), B_w1, B_w2, B_w3, B_w4)
    return out.reshape(1, S, D)
```

```python
import functools

import jax
import jax.numpy as jnp
import jax.experimental.pallas as pl
import jax.experimental.pallas.tpu as pltpu

F32 = jnp.float32
BF16 = jnp.bfloat16

S, D, H, DH, M, SEG, FF = 2048, 640, 32, 192, 8, 32, 1536
NSEG = S // SEG
L = M + SEG
NPAIR = H // 2
PW = 2 * DH
QW = 3 * PW
DT = D // 128
LAG = 3
RING = 4
ZSLOT = RING
NSLOT = RING + 1
HALO = 8
EPS = 1e-5
SCALE = DH ** (-0.5)
NT = (((1,), (1,)), ((), ()))
KPRE = 12
NPRE = KPRE + LAG
RPRE = KPRE * SEG
PIPE = (1, 2, 3, 4)
BPOS_HEAD, BPOS_PRE, BPOS_MAIN, BPOS_LAST, BPOS_TAIL = (
    (4, 8, 12, 16), (4, 6, 8, 10), (2, 4, 6, 8), (2, 4, 7, 10), (10, 13, 15, 17))


def _ln(x):
    m = jnp.mean(x, axis=-1, keepdims=True)
    xc = x - m
    v = jnp.mean(xc * xc, axis=-1, keepdims=True)
    return xc * jax.lax.rsqrt(v + EPS)


def _gelu(x):
    return jax.nn.gelu(x, approximate=True)


def _cat(xs, axis=0):
    return xs[0] if len(xs) == 1 else jnp.concatenate(xs, axis=axis)


def _lhs(x):
    return x.astype(BF16) if x.shape[0] % 16 == 0 else x.astype(F32)


def _mm(a, b):
    return jnp.dot(_lhs(a), b, preferred_element_type=F32)


def _blockdiag(a):
    lane = jax.lax.broadcasted_iota(jnp.int32, (L, 128), 1)
    lo = lane < (DH - 128)
    a0, a1, a2 = a[:, 0:128], a[:, 128:256], a[:, 256:384]
    z = jnp.zeros_like(a0)
    top = jnp.concatenate([a0, jnp.where(lo, a1, 0.0), z], axis=1)
    bot = jnp.concatenate([z, jnp.where(lo, 0.0, a1), a2], axis=1)
    return jnp.concatenate([top, bot], axis=0).astype(BF16)


def _scores(q, k):
    return jax.lax.dot_general(q, _blockdiag(k), NT, preferred_element_type=F32)


def _softmax(s):
    shape = s.shape
    lane = jax.lax.broadcasted_iota(jnp.int32, shape, 1)
    row = jax.lax.broadcasted_iota(jnp.int32, shape, 0) + (L - shape[0])
    h0 = lane < L
    key = jnp.where(h0, lane, lane - L)
    mask = (row < M) | (row >= key)
    s = jnp.where(mask, s * SCALE, -1e9)
    ninf = -jnp.inf
    m0 = jnp.max(jnp.where(h0, s, ninf), axis=-1, keepdims=True)
    m1 = jnp.max(jnp.where(h0, ninf, s), axis=-1, keepdims=True)
    e = jnp.exp(s - jnp.where(h0, m0, m1))
    l0 = jnp.sum(jnp.where(h0, e, 0.0), axis=-1, keepdims=True)
    l1 = jnp.sum(jnp.where(h0, 0.0, e), axis=-1, keepdims=True)
    return e / jnp.where(h0, l0, l1)


def _pv(p, v):
    return jnp.dot(p, _blockdiag(v), preferred_element_type=F32)


def _shift_mix(win):
    lane = jax.lax.broadcasted_iota(jnp.int32, (SEG, 128), 1)

    def sh(tile, off):
        return win[HALO + off:HALO + off + SEG, tile * 128:(tile + 1) * 128]
    c = D // 4
    return jnp.concatenate([
        sh(0, -1),
        jnp.where(lane < c - 128, sh(1, -1), sh(1, 1)),
        jnp.where(lane < 2 * c - 256, sh(2, 1), sh(2, -2)),
        jnp.where(lane < 3 * c - 384, sh(3, -2), sh(3, 2)),
        sh(4, 2)], axis=1)


def _static(t):
    return isinstance(t, int)


def _rows(slot, n=SEG, off=0, unit=SEG):
    if _static(slot):
        return pl.ds(slot * SEG + off, n)
    return pl.ds(pl.multiple_of(slot * SEG + off, unit), n)


def _ring(s):
    return s & (RING - 1)


def inner_kernel(x_hbm, mem0_ref, wq_hbm, wk_hbm, wv_hbm, wo_hbm,
                 w1_hbm, w2_hbm, w3_hbm, w4_hbm,
                 out_hbm,
                 wtq, wtk, wtv, wn, wo, w1, w2, w3, w4,
                 x0, lp, ub, pre, m0y, x1, x2, x3, z1, z2, h1, h2, mem, obuf,
                 qsem, sems):

    def blk(i, n, unit):
        return pl.ds(i * n if _static(i) else pl.multiple_of(i * n, unit), n)

    def qkv_copies(p):
        r = blk(p, PW, 128)
        return [pltpu.make_async_copy(a.at[r, :], b.at[r, :], qsem.at[p & 3])
                for a, b in ((wq_hbm, wtq), (wk_hbm, wtk), (wv_hbm, wtv))]

    def wo_copy(p):
        r = blk(p, PW, 128)
        return pltpu.make_async_copy(wo_hbm.at[r, :], wo.at[r, :], sems.at[2])

    bws = ((w1_hbm, w1), (w2_hbm, w2), (w3_hbm, w3), (w4_hbm, w4))

    def b_copy(j, i):
        a, b = bws[j]
        r = blk(i, b.shape[0] // 4, 16)
        return pltpu.make_async_copy(a.at[r, :], b.at[r, :], sems.at[3 + j])

    hd = NPRE * SEG
    xh = pltpu.make_async_copy(x_hbm.at[pl.ds(0, hd), :], x0.at[pl.ds(0, hd), :], sems.at[0])
    xt = pltpu.make_async_copy(x_hbm.at[pl.ds(hd, S - hd), :], x0.at[pl.ds(hd, S - hd), :],
                               sems.at[1])
    xh.start()
    for cp in qkv_copies(0):
        cp.start()

    zero = jnp.zeros((SEG, D), F32)
    for b in (h1, h2):
        b[_rows(ZSLOT), :] = zero
    m0 = mem0_ref[...].astype(F32)
    mem[pl.ds(0, M), :] = m0
    mem[pl.ds(M, M), :] = m0

    xh.wait()
    for cp in qkv_copies(1):
        cp.start()
    wo_copy(0).start()
    b_copy(0, 0).start()
    lp[...] = _ln(x0[pl.ds(0, RPRE), :].astype(F32)).astype(BF16)

    def pre_body(p, c):
        for cp in qkv_copies(p):
            cp.wait()

        @pl.when(p + 2 < NPAIR)
        def _():
            for cp in qkv_copies(p + 2):
                cp.start()

        @pl.when(p + 1 < NPAIR)
        def _():
            wo_copy(p + 1).start()
        for j in range(4):
            @pl.when((p + 1 < NPAIR) & ((p + 1) // 4 == j))
            def _():
                b_copy(j, (p + 1) % 4).start()
        r = blk(p, PW, 128)
        w = jnp.concatenate([wtq[r, :], wtk[r, :], wtv[r, :]], axis=0)
        wt = w.T
        for c_ in range(QW // 128):
            wn[p, c_, :, :] = wt[:, c_ * 128:(c_ + 1) * 128]
        y = jax.lax.dot_general(lp[...], w, NT, preferred_element_type=F32)
        pre[p, pl.ds(0, RPRE), :] = y.astype(BF16)
        return c

    jax.lax.fori_loop(0, NPAIR, pre_body, 0)
    xt.start()
    pltpu.make_async_copy(wo_hbm, wo, sems.at[2]).wait()
    for j, (a, b) in enumerate(bws):
        pltpu.make_async_copy(a, b, sems.at[3 + j]).wait()

    def ub_load(i):
        return jnp.concatenate([ub[c, pl.ds(i * SEG, SEG), :] for c in range(DT)], axis=1)

    def ub_store(i, val, stores):
        v = val.astype(BF16)
        for c in range(DT):
            stores.append((ub, (c, pl.ds(i * SEG, SEG)), v[:, c * 128:(c + 1) * 128]))

    def wcols(p, lo, hi):
        return jnp.concatenate([wn[p, c] for c in range(lo, hi)], axis=1)

    def a_stage(t, a1, a2, stores):
        last1 = _static(t) and t == NSEG - 1
        last2 = _static(t) and t - LAG == NSEG - 1
        res, toks = [], []
        if a1:
            res.append(x0[_rows(t), :].astype(F32))
            if a1 != "pre":
                toks.append(ub_load(0))
            if a1 == "ahead" and t + 1 < LAG:
                ub_store(0, _ln(x0[_rows(t + 1 + KPRE), :].astype(F32)), stores)
            if a1 == "now" and not last1:
                ub_store(0, _ln(x0[_rows(t + 1), :].astype(F32)), stores)
        if a2:
            res.append(x2[_rows(_ring(t - LAG)), :])
            toks.append(ub_load(1))
        first2 = _static(t) and t == LAG
        if first2:
            h = jnp.concatenate([mem[pl.ds(0, M), :], toks[0].astype(F32)], axis=0)
            m1, t2 = 0, M
        elif a1 and a2:
            h = jnp.concatenate([mem[...].astype(BF16)] + toks, axis=0)
            m1, m2, t1 = 0, M, 2 * M
            t2 = t1 + (SEG if a1 == "now" else 0)
        else:
            h = jnp.concatenate([mem[pl.ds(0 if a1 else M, M), :], toks[0].astype(F32)], axis=0)
            m1 = m2 = 0
            t1 = t2 = M
        hq = _lhs(h[M:]) if (last1 or last2) else None

        def project(p):
            if hq is None:
                y = jnp.dot(h, wcols(p, 0, 9), preferred_element_type=F32)
                return y[:, 0:PW], y[:, PW:2 * PW], y[:, 2 * PW:]
            yq = jnp.dot(hq, wcols(p, 0, 3), preferred_element_type=F32)
            y = jnp.dot(h, wcols(p, 3, 9), preferred_element_type=F32)
            return yq, y[:, 0:PW], y[:, PW:]

        def split(yj, p, j):
            qo = M if (j == 0 and hq is not None) else 0
            out = []
            if a1:
                if a1 == "now":
                    tok = yj[t1 - qo:t1 - qo + SEG]
                else:
                    tok = pre[p, _rows(t), pl.ds(j * PW, PW)].astype(F32)
                out.append(tok if (j == 0 and last1)
                           else jnp.concatenate([yj[m1:m1 + M], tok], axis=0))
            if a2:
                tok = yj[t2 - qo:t2 - qo + SEG]
                if first2:
                    out.append(jnp.concatenate([m0y[p, :, pl.ds(j * PW, PW)], tok], axis=0))
                elif j == 0 and last2:
                    out.append(tok)
                else:
                    out.append(jnp.concatenate([yj[m2 - qo:m2 - qo + M], tok], axis=0))
            return out

        acc = None
        y, s, pr, o = {}, {}, {}, {}
        d1, d2, d3, d4 = PIPE
        for j in range(NPAIR + d4):
            if j < NPAIR:
                y[j] = project(j)
                if a1 == "ahead":
                    pre[j, _rows(t + KPRE), :] = jnp.concatenate(
                        [a[t1:t1 + SEG] for a in y[j]], axis=1).astype(BF16)
                    if t == 0:
                        m0y[j] = jnp.concatenate([a[0:M] for a in y[j]], axis=1)
            p = j - d1
            if 0 <= p < NPAIR:
                s[p] = [_scores(q, k) for q, k in zip(split(y[p][0], p, 0), split(y[p][1], p, 1))]
            p = j - d2
            if 0 <= p < NPAIR:
                pr[p] = [_softmax(a) for a in s.pop(p)]
            p = j - d3
            if 0 <= p < NPAIR:
                o[p] = _cat([_pv(a, v) for a, v in zip(pr.pop(p), split(y.pop(p)[2], p, 2))])
            p = j - d4
            if 0 <= p < NPAIR:
                d = _mm(o.pop(p), wo[pl.ds(p * PW, PW), :])
                acc = d if acc is None else acc + d
            yield
        r = 0
        if a1:
            if not last1:
                stores.append((mem, (pl.ds(0, M),), acc[0:M]))
                r = M
            stores.append((x1, (_rows(_ring(t)),), res[0] + acc[r:r + SEG]))
            r += SEG
        if a2:
            if not last2:
                stores.append((mem, (pl.ds(M, M),), acc[r:r + M]))
                r += M
            stores.append((x3, (_rows(_ring(t - LAG)),), res[-1] + acc[r:r + SEG]))

    def bb_chain(sh, zz, xres):
        g = _mm(_cat(sh), w2[...])
        yield
        y1 = _cat(zz) + g
        g = _mm(_ln(y1), w3[...])
        yield
        g = _mm(_gelu(g), w4[...])
        yield
        yield _cat(xres) + (y1 + g)

    def prev_tail(href, s):
        if _static(s):
            slot = ZSLOT if s == 0 else _ring(s - 1)
        else:
            slot = jnp.where(s == 0, ZSLOT, _ring(s - 1))
        return href[_rows(slot, HALO, SEG - HALO, HALO), :]

    def b_stage(t, b1, b2, stores):
        lay = [(x1, z1, h1, t - 1, x2, b1), (x3, z2, h2, t - 1 - LAG, None, b2)]
        ba = [i for i, l in enumerate(lay) if l[5][0]]
        bb = [i for i, l in enumerate(lay) if l[5][1]]
        head = {}
        zv = {}
        for i in set(ba) & set(bb):
            if not _static(t):
                zv[i] = lay[i][1].at[_rows(lay[i][3] - 1, 2 * SEG), :]
        if ba:
            z = _ln(_cat([lay[i][0][_rows(_ring(lay[i][3])), :] for i in ba]))
            g = _mm(_ln(z), w1[...])
        yield
        if ba:
            hh = _gelu(g)
            for n, i in enumerate(ba):
                _, zr, hr, s, _, _ = lay[i]
                hi = hh[n * SEG:(n + 1) * SEG]
                head[i] = hi[0:HALO]
                if i in zv:
                    zv[i][pl.ds(SEG, SEG), :] = z[n * SEG:(n + 1) * SEG]
                else:
                    zr[_rows(s), :] = z[n * SEG:(n + 1) * SEG]
                stores.append((hr, (_rows(_ring(s)),), hi))
        if not bb:
            return
        sh, zz, xres = [], [], []
        for i in bb:
            xr, zr, hr, s, _, _ = lay[i]
            s = s - 1
            nxt = head[i] if i in head else jnp.zeros((HALO, D), F32)
            sh.append(_shift_mix(jnp.concatenate(
                [prev_tail(hr, s), hr[_rows(_ring(s)), :], nxt], axis=0)))
            zz.append(zv[i][pl.ds(0, SEG), :] if i in zv else zr[_rows(s), :])
            xres.append(xr[_rows(_ring(s)), :])
        chain = bb_chain(sh, zz, xres)
        for _ in range(3):
            next(chain)
            yield
        xn = next(chain)
        for n, i in enumerate(bb):
            s = lay[i][3] - 1
            v = xn[n * SEG:(n + 1) * SEG]
            if lay[i][4] is not None:
                stores.append((lay[i][4], (_rows(_ring(s)),), v))
                ub_store(1, _ln(v), stores)
            else:
                stores.append((obuf, (_rows(s),), v.astype(BF16)))

    def step(t, a1, a2, b1, b2, bpos):
        stores = []
        bg = b_stage(t, b1, b2, stores)
        for j, _ in enumerate(a_stage(t, a1, a2, stores)):
            if j in bpos:
                next(bg, None)
        for _ in bg:
            pass
        for ref, idx, val in stores:
            ref[idx + (slice(None),)] = val

    def auto(t, a1, bpos):
        ok = lambda s: 0 <= s < NSEG
        step(t, a1 if ok(t) else None, ok(t - LAG),
             (ok(t - 1), ok(t - 2)), (ok(t - 1 - LAG), ok(t - 2 - LAG) and t < NSEG + LAG - 1),
             bpos)

    def loop(lo, hi, a1, bpos):
        def body(t, c):
            step(t, a1, True, (True, True), (True, True), bpos)
            return c
        jax.lax.fori_loop(lo, hi, body, 0)

    def prefill(seg):
        st = []
        ub_store(0, _ln(x0[_rows(seg), :].astype(F32)), st)
        for ref, idx, val in st:
            ref[idx + (slice(None),)] = val

    def out_copy(lo, hi, i):
        r = pl.ds(lo * SEG, (hi - lo) * SEG)
        return pltpu.make_async_copy(obuf.at[r, :], out_hbm.at[r, :], sems.at[i])

    prefill(KPRE)
    for t in range(LAG):
        auto(t, "ahead", BPOS_HEAD)
    for t in range(LAG, LAG + 2):
        auto(t, "pre", BPOS_PRE)
    loop(LAG + 2, NPRE, "pre", BPOS_PRE)
    xt.wait()
    prefill(NPRE)
    loop(NPRE, NSEG - 1, "now", BPOS_MAIN)
    auto(NSEG - 1, "now", BPOS_LAST)
    done = NSEG - 5
    out_copy(0, done, 0).start()
    for t in range(NSEG, NSEG + LAG):
        auto(t, None, BPOS_TAIL)

    sa, sb, sc = NSEG - 1, NSEG - 2, NSEG - 3
    xa, xb, xc = [x3[_rows(_ring(s)), :] for s in (sa, sb, sc)]
    hb, hc = h2[_rows(_ring(sb)), :], h2[_rows(_ring(sc)), :]
    side = bb_chain([_shift_mix(jnp.concatenate([prev_tail(h2, sc), hc, hb[0:HALO]], axis=0))],
                    [z2[_rows(sc), :]], [xc])
    za = _ln(xa)
    g = _mm(_ln(za), w1[...])
    next(side)
    ha = _gelu(g)
    winb = jnp.concatenate([hc[SEG - HALO:], hb, ha[0:HALO]], axis=0)
    wina = jnp.concatenate([hb[SEG - HALO:], ha, jnp.zeros((HALO, D), F32)], axis=0)
    chain = bb_chain([_shift_mix(winb), _shift_mix(wina)], [z2[_rows(sb), :], za], [xb, xa])
    for c in (chain, side, chain, side, chain):
        next(c)
    obuf[_rows(sc), :] = next(side).astype(BF16)
    obuf[_rows(sb, 2 * SEG), :] = next(chain).astype(BF16)

    out_copy(done, NSEG, 1).start()
    out_copy(0, done, 0).wait()
    out_copy(done, NSEG, 1).wait()


@functools.partial(jax.jit, static_argnames=("A_seg_len",))
def pallas_interleave_layers__memory_aug_recurrent_mem_tr__mixer_s_mlp__prompt_kernel(
    A_x, A_mem0, A_Wq, A_Wk, A_Wv, A_Wo, A_seg_len, B_x, B_w1, B_w2, B_w3, B_w4,
):
    del B_x
    assert A_seg_len == SEG and A_x.shape == (1, S, D) and A_mem0.shape == (1, M, D)
    assert A_Wq.shape == (D, H, DH) and A_Wo.shape == (H, DH, D) and B_w3.shape == (D, FF)

    def wt(w):
        return jnp.transpose(w, (1, 2, 0)).reshape(H * DH, D)

    any_spec = pl.BlockSpec(memory_space=pl.ANY)
    ring = pltpu.VMEM((RING * SEG, D), F32)
    out = pl.pallas_call(
        inner_kernel,
        out_shape=jax.ShapeDtypeStruct((S, D), BF16),
        in_specs=[any_spec, pl.BlockSpec(memory_space=pltpu.VMEM)] + [any_spec] * 8,
        out_specs=any_spec,
        scratch_shapes=[
            pltpu.VMEM((H * DH, D), BF16),
            pltpu.VMEM((H * DH, D), BF16),
            pltpu.VMEM((H * DH, D), BF16),
            pltpu.VMEM((NPAIR, QW // 128, D, 128), BF16),
            pltpu.VMEM((H * DH, D), BF16),
            pltpu.VMEM((D, D), BF16),
            pltpu.VMEM((D, D), BF16),
            pltpu.VMEM((D, FF), BF16),
            pltpu.VMEM((FF, D), BF16),
            pltpu.VMEM((S, D), BF16),
            pltpu.VMEM((RPRE, D), BF16),
            pltpu.VMEM((DT, 2 * SEG, 128), BF16),
            pltpu.VMEM((NPAIR, NPRE * SEG, QW), BF16),
            pltpu.VMEM((NPAIR, M, QW), F32),
            ring, ring, ring,
            pltpu.VMEM((S, D), F32), pltpu.VMEM((S, D), F32),
            pltpu.VMEM((NSLOT * SEG, D), F32),
            pltpu.VMEM((NSLOT * SEG, D), F32),
            pltpu.VMEM((2 * M, D), F32),
            pltpu.VMEM((S, D), BF16),
            pltpu.SemaphoreType.DMA((4,)),
            pltpu.SemaphoreType.DMA((7,)),
        ],
        compiler_params=pltpu.CompilerParams(vmem_limit_bytes=120 * 2**20,
                                             disable_bounds_checks=True),
    )(A_x.reshape(S, D), A_mem0.reshape(M, D), wt(A_Wq), wt(A_Wk), wt(A_Wv),
      A_Wo.reshape(H * DH, D), B_w1, B_w2, B_w3, B_w4)
    return out.reshape(1, S, D)
```
